```python
import jax
import jax.numpy as jnp

def _softmax(x, axis=-1):
    return jax.nn.softmax(x, axis=axis)
def _gelu(x):
    return jax.nn.gelu(x, approximate=True)
def _silu(x):
    return jax.nn.silu(x)
def _sigmoid(x):
    return jax.nn.sigmoid(x)
def _layernorm(x, axis=-1, eps=1e-5):
    m = jnp.mean(x, axis=axis, keepdims=True)
    v = jnp.var(x, axis=axis, keepdims=True)
    return (x - m) / jnp.sqrt(v + eps)
def _scatter_add(tgt, idx, src, axis=0):
    return tgt.at[idx].add(src)
def _segment_sum(src, seg, n):
    return jax.ops.segment_sum(src, seg, n)
class _Rng:
    def __init__(self, key):
        self._k = key
    def _next(self):
        self._k, sub = jax.random.split(self._k)
        return sub
    def normal(self, shape):
        return jax.random.normal(self._next(), shape, dtype=jnp.bfloat16)
    def randint(self, lo, hi, shape):
        return jax.random.randint(self._next(), shape, lo, hi, dtype=jnp.int32)
    def uniform(self, shape, lo=0.0, hi=1.0):
        return jax.random.uniform(self._next(), shape, jnp.bfloat16, lo, hi)
    def permutation(self, n):
        return jax.random.permutation(self._next(), n)


kernel_name = 'standalone__dcn_v2_cross__recsys'

def setup_inputs():
    _rng = _Rng(jax.random.key(int.from_bytes(__import__("os").urandom(4), "little")))
    _w = (lambda a: (lambda t: t.astype(jnp.bfloat16) if jnp.issubdtype(t.dtype, jnp.floating) else t)(jnp.asarray(a)))
    B, F, D, L = 16384, 26, 128, 6
    Din = min(F * D, 1024)
    return {
        "x0": _w((lambda *s: _rng.normal(s) * 0.05)(B, Din)),
        "ws": _w((lambda *s: _rng.normal(s) * 0.05)(L, Din, Din)),
        "bs": _w((lambda *s: _rng.normal(s) * 0.05)(L, Din)),
    }

def reference(x0, ws, bs):
    x = x0
    for l in range(ws.shape[0]):
        x = x0 * (x @ ws[l] + bs[l]) + x
    return x
```

```python
import functools

import jax
import jax.numpy as jnp
import jax.experimental.pallas as pl
import jax.experimental.pallas.tpu as pltpu


def _kernel(x0_ref, ws_ref, bs_ref, o_ref, *, n_layers):
    x0 = x0_ref[...].astype(jnp.float32)
    x = x0
    for l in range(n_layers):
        y = jnp.dot(x.astype(jnp.bfloat16), ws_ref[l],
                    preferred_element_type=jnp.float32)
        x = x0 * (y + bs_ref[l].astype(jnp.float32)) + x
    o_ref[...] = x.astype(o_ref.dtype)


@jax.jit
def pallas_standalone__dcn_v2_cross__recsys_kernel(
    x0: jax.Array,
    ws: jax.Array,
    bs: jax.Array,
):
    B, D = x0.shape
    L = ws.shape[0]
    tm = 512
    bs3 = bs.reshape(L, 1, D)
    return pl.pallas_call(
        functools.partial(_kernel, n_layers=L),
        grid=(B // tm,),
        in_specs=[
            pl.BlockSpec((tm, D), lambda i: (i, 0)),
            pl.BlockSpec((L, D, D), lambda i: (0, 0, 0)),
            pl.BlockSpec((L, 1, D), lambda i: (0, 0, 0)),
        ],
        out_specs=pl.BlockSpec((tm, D), lambda i: (i, 0)),
        out_shape=jax.ShapeDtypeStruct((B, D), x0.dtype),
        compiler_params=pltpu.CompilerParams(
            dimension_semantics=("arbitrary",),
            vmem_limit_bytes=100 * 1024 * 1024,
        ),
    )(x0, ws, bs3)
```

```python
import functools
import jax
import jax.numpy as jnp
import jax.experimental.pallas as pl
import jax.experimental.pallas.tpu as pltpu

F32 = jnp.float32
BF16 = jnp.bfloat16

LA = [{0: 1, 3: 1}, {2: 1, 3: 1}, {0: 1}, {3: 1}, {0: 1, 1: 1}, {2: 1, 0: -1}, {1: 1, 3: -1}]
LB = [{0: 1, 3: 1}, {0: 1}, {1: 1, 3: -1}, {2: 1, 0: -1}, {3: 1}, {0: 1, 1: 1}, {2: 1, 3: 1}]
M1, M2, M3, M4, M5, M6, M7 = range(7)


def lin(terms):
    k = next(i for i, t in enumerate(terms) if t[0] > 0)
    acc = terms[k][1]
    for i, (c, v) in enumerate(terms):
        if i != k:
            acc = acc + v if c > 0 else acc - v
    return acc


def _quads(a):
    m, k = a.shape
    return [a[:m // 2, :k // 2], a[:m // 2, k // 2:], a[m // 2:, :k // 2], a[m // 2:, k // 2:]]


def _b_ops(b, lev):
    if lev == 0:
        return [b]
    q = _quads(b)
    out = []
    for i in range(7):
        out += _b_ops(lin([(c, q[j]) for j, c in LB[i].items()]), lev - 1)
    return out


X = [0, 16]
R2, R3, P, K12, K21 = 32, 36, 40, 44, 48
TMP = 52
NTMP = 6
NSLOT = TMP + 2 * NTMP


def layer_program():
    prog = []
    g = [0]

    def tmps():
        b = TMP + (g[0] % 2) * NTMP
        g[0] += 1
        return [b + k for k in range(NTMP)]

    def temp_phase(I, acc, dst):
        a = lambda e: [(c, s + e) for c, s in acc]
        r4, r5, r7 = tmps()[:3]
        prog.append((I, M4, [(1, [], r4, None)]))
        prog.append((I, M7, [(1, [], r7, None)]))
        prog.append((I, M2, [(1, [(1, r4)] + a(2), dst + 2, None)]))
        prog.append((I, M5, [(1, [], r5, None)]))
        prog.append((I, M6, [(1, [(-1, r7)] + a(3), dst + 3, None)]))
        prog.append((I, M3, [(1, [(1, r5)] + a(1), dst + 1, None)]))
        prog.append((I, M1, [(1, [(1, r4), (-1, r5), (1, r7)] + a(0), dst + 0, None)]))

    def final_phase(I, acc, CQ, dst):
        a = lambda e: [(c, s + e) for c, s in acc]
        r2, r3, p, c12, c21, t = tmps()
        if dst is not None:
            c12, c21 = dst + 1, dst + 2
        prog.append((I, M2, [(1, a(2), r2, None)]))
        prog.append((I, M3, [(1, a(1), r3, None)]))
        prog.append((I, M1, [(1, [(1, r3), (-1, r2)] + a(0), p, None)]))
        o = [(1, a(3) + [(1, p)], None, (CQ, 3))]
        if dst is not None:
            o.append((1, a(3), t, None))
        prog.append((I, M6, o))
        prog.append((I, M5, [(1, [(1, r3)], c12, (CQ, 1))]))
        prog.append((I, M4, [(1, [(1, r2)], c21, (CQ, 2))]))
        o = [(1, [(1, p), (1, c21), (-1, c12)], dst, (CQ, 0))]
        if dst is not None:
            o.append((-1, [(1, t)], dst + 3, None))
        prog.append((I, M7, o))

    temp_phase(M2, [], R2)
    temp_phase(M3, [], R3)
    temp_phase(M1, [(1, R3), (-1, R2)], P)
    final_phase(M6, [(1, P)], 3, None)
    final_phase(M5, [(1, R3)], 1, K12)
    final_phase(M4, [(1, R2)], 2, K21)
    final_phase(M7, [(1, P), (1, K21), (-1, K12)], 0, None)
    return prog


def _kernel(x0_ref, ws_ref, bs_ref, o_ref, t_ref, z_ref, buf_ref, *, n_layers, tm, mode):
    D = x0_ref.shape[1]
    rm, rk = tm // 4, D // 4

    @pl.when(pl.program_id(0) == 0)
    def _():
        z_ref[0] = 0
        def body(l, c):
            ops = _b_ops(ws_ref[l].astype(F32), 2)
            for i, o in enumerate(ops):
                t_ref[l, i] = pltpu.bitcast(o.astype(BF16), jnp.uint32)
            return c
        jax.lax.fori_loop(0, n_layers, body, 0)

    buf = buf_ref.at[z_ref[0]]

    def blk(Q, q):
        r = (Q // 2) * 2 + q // 2
        c = (Q % 2) * 2 + q % 2
        return r * rm, c * rk

    def x0blk(Q, q):
        r, c = blk(Q, q)
        return x0_ref[r:r + rm, c:c + rk].astype(F32)

    prog = layer_program()
    for l in range(n_layers):
        def xblk(Q, q):
            if l == 0:
                return x0blk(Q, q)
            return buf[X[l % 2] + Q * 4 + q]

        for I, i, outs in prog:
            a = lin([(c * C, xblk(J, j)) for j, c in LA[i].items() for J, C in LA[I].items()])
            w = pltpu.bitcast(t_ref[l, I * 7 + i], BF16)
            m = jnp.dot(a.astype(BF16), w, preferred_element_type=F32)
            for cm, terms, dst, epi in outs:
                if mode == 0:
                    y = lin([(cm, m)] + [(c, buf[s]) for c, s in terms])
                else:
                    y = lin([(c, buf[s]) for c, s in terms] + [(cm, m)])
                if dst is not None:
                    buf[dst] = y
                if epi is not None:
                    CQ, cq = epi
                    r, c = blk(CQ, cq)
                    b = bs_ref[l:l + 1, c:c + rk].astype(F32)
                    v = x0blk(CQ, cq) * (y + b) + xblk(CQ, cq)
                    if l == n_layers - 1:
                        o_ref[r:r + rm, c:c + rk] = v.astype(o_ref.dtype)
                    else:
                        buf[X[(l + 1) % 2] + CQ * 4 + cq] = v


@jax.jit
def pallas_standalone__dcn_v2_cross__recsys_kernel(x0, ws, bs):
    tm, mode, lead = 512, 0, 1
    B, D = x0.shape
    L = ws.shape[0]
    d = D // 4
    return pl.pallas_call(
        functools.partial(_kernel, n_layers=L, tm=tm, mode=mode),
        grid=(B // tm,),
        in_specs=[
            pl.BlockSpec((tm, D), lambda i: (i, 0)),
            pl.BlockSpec((L, D, D), lambda i: (0, 0, 0), pipeline_mode=pl.Buffered(1)),
            pl.BlockSpec((L, D), lambda i: (0, 0)),
        ],
        out_specs=pl.BlockSpec((tm, D), lambda i: (i, 0)),
        out_shape=jax.ShapeDtypeStruct((B, D), x0.dtype),
        scratch_shapes=[pltpu.VMEM((L, 49, d // 2, d), jnp.uint32), pltpu.SMEM((1,), jnp.int32),
                        pltpu.VMEM((lead, NSLOT, tm // 4, d), F32)],
        compiler_params=pltpu.CompilerParams(
            dimension_semantics=("arbitrary",),
            vmem_limit_bytes=120 * 1024 * 1024,
        ),
    )(x0, ws, bs)
```

```python
import functools
import numpy as np
import jax
import jax.numpy as jnp
import jax.experimental.pallas as pl
import jax.experimental.pallas.tpu as pltpu

F32 = jnp.float32
BF16 = jnp.bfloat16
U32 = jnp.uint32
M1, M2, M3, M4, M5, M6, M7 = range(7)
SQ3 = float(np.sqrt(3.0))
LAM = [1.0, 1 / SQ3, SQ3, 1.0]
RL = 64
HALF = 4 * RL
AOP = {M1: [(1, 0)], M3: [(1, 1)], M4: [(1, 0), (-1, 1)], M5: [(1, 2)], M7: [(1, 0), (-1, 2)], M2: [(1, 3)], M6: [(1, 0), (-1, 3)]}
BOP = {M1: [(1, 0)], M2: [(1, 1)], M5: [(1, 0), (-1, 1)], M6: [(1, 2)], M3: [(1, 0), (-1, 2)], M7: [(1, 3)], M4: [(1, 0), (-1, 3)]}
BOP_OUT = {M1: [(1, 4)], M2: [(1, 1)], M5: [(1, 0), (-1, 1)], M6: [(1, 2)], M3: [(1, 0), (-1, 2)], M7: [(1, 3)], M4: [(1, 4), (-1, 3)]}
PRIMED = [M5, M2, M6]
FIN = {M1: (0, -1, [(1, M5), (1, M2), (1, M6)]), M4: (1, 1, [(-1, M2)]), M7: (2, 1, [(-1, M6)]), M3: (3, 1, [(-1, M5)])}

_n = [0]
def _it(k=1):
    r = list(range(_n[0], _n[0] + k)); _n[0] += k
    return r
SS = _it(2)
GP, GM, NN, PP, TR, UP, UM = (_it()[0] for _ in range(7))
TMP = _it(2)
X0 = _it(4)
YY = _it(4)
_a = _it(15)
_z = _it(8)
R3, R5 = [_a[0], _a[0]], [_a[1], _a[1]]
HH, R4, R7, R2, R6 = ([_a[2 + k], _z[k]] for k in range(5))
DD = [_a[7], _a[8], _z[5]]
C11 = [_a[9], _a[10], _a[10]]
C22 = [_z[6], _a[11], _a[12]]
ZZ = [_z[7], _a[13], _a[14]]
NI = _n[0]
SG = RL + 8
SF = 4 * SG + 8
SI = 4 * SF + 8
WG = 128 + 8
WF = 4 * WG + 8
WI = 4 * WF + 8
assert 10 * WI <= _z[0] * SI


def lin(terms):
    k = next(i for i, t in enumerate(terms) if t[0] > 0)
    acc = terms[k][1]
    for i, (c, v) in enumerate(terms):
        if i != k:
            acc = acc + v if c > 0 else acc - v
    return acc


def a_tr(a11, s, t, a22):
    tr = a11 + a22
    return [tr, a11 - s, a11 + s, (tr + (s + t)) * 0.5]


def c_tr(e0, e1, e2, e3, half=0.5):
    h = e3 * half
    c22 = e0 + h
    return [(c22 + e1) + e2, h, (h + e1) - e2, c22]


class Item:
    def __init__(self, key, cost, rel, dl, preds, fn):
        self.key, self.cost, self.rel, self.dl, self.preds, self.fn, self.pos = key, cost, rel, dl, preds, fn, None


def water(fixed, free, a, b, work):
    f = np.sort(fixed[a:b][free[a:b]])
    if len(f) == 0:
        return np.inf
    lv = (work + np.cumsum(f)) / np.arange(1, len(f) + 1)
    return lv[np.nonzero(lv >= f)[0][-1]]


def place(items, fixed, lat, slack):
    n = len(fixed)
    jobs = {}
    for it in items:
        k = (int(np.ceil(it.rel)), int(np.floor(it.dl)))
        jobs[k] = jobs.get(k, 0.0) + it.cost
    free = np.ones(n, bool)
    room = np.zeros(n)
    while jobs:
        best = None
        for a in sorted({k[0] for k in jobs}):
            for b in sorted({k[1] for k in jobs}):
                w = sum(v for k, v in jobs.items() if k[0] >= a and k[1] <= b)
                if b > a and w > 0:
                    lv = water(fixed, free, a, b, w)
                    if best is None or lv > best[0]:
                        best = (lv, a, b)
        lv, a, b = best
        idx = np.arange(a, b)[free[a:b]]
        room[idx] = np.maximum(lv - fixed[idx], 0)
        free[a:b] = False
        jobs = {k: v for k, v in jobs.items() if not (k[0] >= a and k[1] <= b)}
    room = room * slack
    todo = sorted(range(len(items)), key=lambda k: (items[k].dl, k))
    debt = 0.0
    for g in range(n):
        used = debt
        r = room[g]
        while todo and (used < r or items[todo[0]].dl <= g + 1):
            t = g + min(used / max(r, 1e-9), 0.99)
            pick = None
            for j in range(min(len(todo), 400)):
                it = items[todo[j]]
                if it.rel <= t and all(p.pos is not None and (p.pos + lat <= t or used >= r) for p in it.preds):
                    pick = j
                    break
            if pick is None:
                assert used < r
                used += r / 16
                continue
            it = items[todo.pop(pick)]
            it.pos = t
            used += it.cost
        debt = max(used - r, 0.0)
    assert not todo


def _kernel(xc_ref, xp_ref, xl_ref, ws_hbm, bs_ref, o_ref, z_ref, buf_ref, t_ref, bt_ref, w_ref, xf_ref, sav_ref, sem, *,
            morder, lorder, shift, ak, delay, w0, lat, slack, only, fb, afb, pw, pk):
    step = pl.program_id(0)
    nsteps = pl.num_programs(0)
    L = bs_ref.shape[0]
    D = xc_ref.shape[1]

    @pl.when(step == 0)
    def _():
        z_ref[0] = 0

    z0 = z_ref[0]
    buf = buf_ref.at[z0]
    if pk == 3:
        tb = t_ref
        tu = t_ref.bitcast(U32)
        tix = lambda l, n: (l, n)
    else:
        tb = t_ref.bitcast(BF16)
        tix = lambda l, n: (l, n // 2, slice(None), pl.ds((n % 2) * 128, 128))

    def anchored(v, tok):
        if tok is None:
            return v
        return jnp.where(jnp.full(tok.shape, z0, jnp.int32) == 0, v, tok)

    def sl(it, f, g):
        return pl.ds(it * SI + f * SF + g * SG, RL)

    def bits(Q, q, p):
        return (Q // 2) * 4 + (q // 2) * 2 + p // 2, (Q % 2) * 4 + (q % 2) * 2 + p % 2

    def io_idx(Q, q, p):
        r, c = bits(Q, q, p)
        return pl.ds((r ^ 4) * RL, RL), pl.ds(c * 128, 128)

    def put_f(Q, f, g, v, par):
        if Q == 1:
            buf[sl(SS[par], f, g)] = v
            return
        s = buf[sl(SS[par], f, g)]
        if Q == 0:
            buf[sl(NN, f, g)] = v - s
            buf[sl(PP, f, g)] = v + s
        elif Q == 3:
            up = v + s
            buf[sl(TR, f, g)] = up + buf[sl(NN, f, g)]
            buf[sl(UP, f, g)] = up
            buf[sl(UM, f, g)] = v - s
        else:
            w = v + s
            tr = buf[sl(TR, f, g)]
            buf[sl(GP, f, g)] = tr + w
            buf[sl(GM, f, g)] = tr - w
    LCOST = {0: (15, 8, 8), 1: (7, 4, 4), 2: (19, 12, 8), 3: (19, 12, 12)}

    def put_y(Q, p, y):
        for f in range(4):
            buf[sl(YY[Q], f, p)] = y[f]

    def pass_init(Q, p, tok):
        xs = []
        for q in range(4):
            lam = LAM[Q] * LAM[q] * LAM[p]
            v = xc_ref[io_idx(Q, q, p)].astype(F32)
            if Q >= 2 or q == 0:
                v = anchored(v, tok)
            if Q >= 2:
                buf[sl(X0[Q], q, p)] = v
            xs.append(v if abs(lam - 1) < 1e-9 else v * lam)
        put_y(Q, p, a_tr(*xs))

    KT = {1: ([(1, R3), (-1, R5)], DD), 0: ([(1, HH), (1, R4), (1, R7)], C11), 3: ([(1, HH), (1, R2), (1, R6)], C22),
          2: ([(1, R4), (-1, R7), (-1, R2), (1, R6)], ZZ)}

    def pass_k(Q, f, l, tok):
        par = l % 2
        terms, dst = KT[Q]
        e = [lin([(c, buf[sl(it[par], f, g)]) for c, it in terms]) for g in range(4)]
        c = c_tr(*e, half=anchored(0.5, tok))
        for p in range(4):
            v = c[p] if l == 0 else c[p] + buf[sl(dst[1 - par], f, p)]
            buf[sl(dst[2 if l == L - 1 else par], f, p)] = v

    def mix_x(Q, p, l, tok):
        par = 2 if l == L - 1 else l % 2
        if Q == 2:
            e = [buf[sl(DD[par], f, p)] + buf[sl(ZZ[par], f, p)] for f in range(4)]
        else:
            e = [buf[sl(KT[Q][1][par], f, p)] for f in range(4)]
        c = c_tr(*e, half=anchored(0.5, tok))
        res = []
        for q in range(4):
            if (Q < 2 and l == 0) or (Q >= 2 and l == L - 1):
                x0 = xp_ref[io_idx(Q, q, p)].astype(F32)
                if Q < 2:
                    x0 = anchored(x0, tok)
                    buf[sl(X0[Q], q, p)] = x0
            else:
                x0 = buf[sl(X0[Q], q, p)]
            r, cb = bits(Q, q, p)
            b = bt_ref[l, bin(r).count("1"), :, pl.ds(cb * 128, 128)]
            res.append((c[q] + jnp.concatenate([b] * (RL // 8), axis=0)) * x0)
        return res

    def pass_m(Q, p, l, tok):
        put_y(Q, p, a_tr(*mix_x(Q, p, l, tok)))

    def pass_l(Q, f, par, tok):
        y = [buf[sl(YY[Q], f, p)] for p in range(4)]
        y[0] = anchored(y[0], tok)
        for g, v in enumerate(a_tr(*y)):
            put_f(Q, f, g, v, par)

    def pass_final(Q, p, l, tok):
        xt = mix_x(Q, p, l, tok)
        for q in range(4):
            lam = LAM[Q] * LAM[q] * LAM[p]
            v = xt[q] if abs(lam - 1) < 1e-9 else xt[q] * (1 / lam)
            o_ref[io_idx(Q, q, p)] = v.astype(o_ref.dtype)

    def use_afb(I, i):
        return afb == 2 or (afb == 1 and (I == M1 or i == M1))

    def group(l, ph, I, src, acc, dst, i):
        tmp = TMP[(l * 7 + ph) % 2]
        fs = [lin([(c, buf[sl(src, f, g)]) for c, f in AOP[i]]) for g in range(4)]
        ops = {}
        if use_afb(I, i):
            ops[M1] = fs[0].astype(BF16)
            r = ops[M1].astype(F32)
            e2 = (r - fs[0]) * 0.5
            fs = [r] + [v + e2 for v in fs[1:]]
        n = {}
        for k in lorder:
            op = ops[k] if k in ops else lin([(c, fs[g]) for c, g in AOP[k]]).astype(BF16)
            w = pltpu.bitcast(tu[tix(l, (I * 7 + i) * 7 + k)], BF16) if pk == 3 else tb[tix(l, (I * 7 + i) * 7 + k)]
            n[k] = jnp.dot(op, w, preferred_element_type=F32)
        e = [None] * 4
        for k, (f, sg, rt) in FIN.items():
            terms = dict([(k, sg)] + [(x, c) for c, x in rt])
            e[f] = lin([(terms[j], n[j]) for j in lorder if j in terms])
        if i in PRIMED:
            for g in range(4):
                buf[sl(tmp, PRIMED.index(i), g)] = e[g]
        else:
            f, sg, rt = FIN[i]
            so = -1 if I == M1 else 1
            for g in range(4):
                terms = [(so * sg, e[g])] + [(so * c, buf[sl(tmp, PRIMED.index(k), g)]) for c, k in rt] + [(1, buf[sl(it, f, g)]) for it in acc]
                if terms[0][0] < 0:
                    j = next(j for j, t in enumerate(terms) if t[0] > 0)
                    terms = [terms[j], terms[0]] + [t for jj, t in enumerate(terms) if jj not in (0, j)]
                buf[sl(dst, f, g)] = lin(terms)
        return [n[k] for k in lorder]

    P = functools.partial
    cost = lambda valu, ld, st: valu / 4 + ld / 3 + st

    def phases(l):
        par = l % 2
        return [(M3, NN, [], R3[par]), (M5, PP, [], R5[par]), (M1, TR, [R3[par], R5[par]], HH[par]), (M4, UP, [], R4[par]),
                (M7, UM, [], R7[par]), (M2, GP, [], R2[par]), (M6, GM, [], R6[par])]

    NS = (343 * L + 3) // 4
    slot_of = lambda G, k: (7 * G + k) // 4

    def fixed_costs():
        ca, cc = np.zeros(NS + 8), np.zeros(NS + 8)
        G = 0
        kpos = {k: j for j, k in enumerate(lorder)}
        for l in range(L):
            for I, src, acc, dst in phases(l):
                for i in morder:
                    T = len(AOP[i])
                    seen = set()
                    x = 8 if use_afb(I, i) else 0
                    for j, k in enumerate(lorder):
                        new = ({g for _, g in AOP[k]} | ({0} if x else set())) - seen
                        seen |= new
                        ca[slot_of(G, j)] += cost(4 + 8 * (len(AOP[k]) - 1) + (8 * (T - 1) + x) * len(new) + (2 * x if 0 in new else 0), 8 + 8 * T * len(new), 0)
                    nr = 0 if i in PRIMED else len(FIN[i][2]) + len(acc)
                    for k, (f, sg, rt) in FIN.items():
                        arr = sorted([kpos[k]] + [kpos[x] for _, x in rt])
                        for j in arr[1:]:
                            cc[slot_of(G, j)] += cost(8, 0, 0)
                        cc[slot_of(G, arr[-1])] += cost(8 * nr, 8 * nr, 8)
                    G += 1
        lo = int(np.floor(shift)); fr = shift - lo
        return cc[:NS] + (1 - fr) * ca[lo:lo + NS] + fr * ca[lo + 1:lo + NS + 1]

    NG = 49 * L
    t_end = lambda G: slot_of(G, 6) + 1
    t_beg = lambda G: min(slot_of(G, 0), NS)
    done_at = {f: morder.index(i) for i, (f, _, _) in FIN.items()}
    PH_DONE = {1: 1, 0: 4, 3: 6, 2: 6}
    PH_USE = {1: 7, 0: 7, 3: 9, 2: 12}

    def build(kind, Q, l, base, reg, rel0=None, dl_end=None):
        io = Q < 2 and l == 0
        rel = [t_end(base + PH_DONE[Q] * 7 + done_at[f]) + w0 for f in range(4)]
        if kind == 'init':
            rel = [rel0] * 4
        dl = dl_end if kind == 'final' else min(slot_of(base + PH_USE[Q] * 7, 0) - delay, NS)
        x = 4 if Q == 2 else 0
        stages = []
        if kind != 'init':
            nt = len(KT[Q][0])
            stages.append(('K', cost(4 * nt + 7, 4 * nt + 4, 4), [P(pass_k, Q, f, l) for f in range(4)]))
        if kind == 'init':
            stages.append(('M', cost(18 if Q >= 2 else 15, 4, 8 if Q >= 2 else 4), [P(pass_init, Q, p) for p in range(4)]))
        elif kind == 'mix':
            stages.append(('M', cost(21 + x + (8 if io else 0), 12 + x, 8 if io else 4), [P(pass_m, Q, p, l) for p in range(4)]))
        else:
            stages.append(('M', cost(22 + x + (4 if Q >= 2 else 0), 12 + x, 4), [P(pass_final, Q, p, l) for p in range(4)]))
        if kind != 'final':
            stages.append(('L', cost(*LCOST[Q]), [P(pass_l, Q, f, (l + 1) % 2) for f in range(4)]))
        items = []
        for t in range(8 + len(stages) - 1):
            for j in range(4):
                for si, (nm, c, fns) in enumerate(stages):
                    r = t - si
                    if not 0 <= r < 8:
                        continue
                    pre = [reg[(stages[si - 1][0], Q, l, jj, r)] for jj in range(4)] if si else []
                    if nm == 'M' and Q == 2:
                        pre += [reg[kk] for kk in [('K', 1, l, f, r) for f in range(4)] if kk in reg]
                    if nm == 'L':
                        pre += [reg[('L', d, l, j, r)] for d in {0: [1], 1: [], 3: [1, 0], 2: [1, 3]}[Q] if ('L', d, l, j, r) in reg]
                    it = Item((nm, Q, l, j, r), c, max(rel[j] if nm == 'K' else max(rel), 0), dl, pre, fns[j])
                    reg[it.key] = it
                    items.append(it)
        return items

    def run_all(items):
        for nm in 'KML':
            for it in items:
                if it.key[0] == nm and it.key[4] == 0:
                    it.fn(None)

    def main_body():
        reg, regp, regn = {}, {}, {}
        items = []
        for Q in (3, 2):
            items += build('init', Q, -1, -49, reg, rel0=0)
        for Q in (3, 2):
            items += build('final', Q, L - 1, -49, regp, dl_end=t_beg(49))
        for it in regp.values():
            if it.key[0] == 'M':
                it.dl = t_beg(49 * (L - 1))
        for l in range(L):
            for Q in (1, 0, 3, 2):
                if l < L - 1:
                    items += build('mix', Q, l, 49 * l, reg)
                elif Q < 2:
                    items += build('final', Q, l, 49 * l, reg, dl_end=NS)
        for Q in (1, 0):
            items += build('init', Q, L - 1, NG, regn, rel0=t_beg(49 * (L - 1)))
        for it in regn.values():
            if it.key[0] == 'L' and it.key[1] == 0:
                it.rel = t_beg(49 * (L - 1) + 14)
        place(items, fixed_costs(), lat, slack)
        batches = {}
        for it in items:
            batches.setdefault(id(it.fn), []).append(it)
            it.prod = min(4 * int(it.pos) + ak, 343 * L - 1)
            it.row = min(int((it.pos - int(it.pos)) * 8), 7)
        blist = sorted(batches.values(), key=lambda b: (max(it.pos for it in b), 'KML'.index(b[0].key[0])))
        toks = []
        k = 0
        for l in range(L):
            for ph, (I, src, acc, dst) in enumerate(phases(l)):
                for i in morder:
                    toks += group(l, ph, I, src, acc, dst, i)
                    while k < len(blist) and max(it.prod for it in blist[k]) < len(toks):
                        b = sorted(blist[k], key=lambda it: it.key[4])
                        b[0].fn(jnp.concatenate([toks[it.prod][8 * it.row:8 * it.row + 8] for it in b], axis=0))
                        k += 1
        assert k == len(blist)

    def wcopy(l, slot):
        return pltpu.make_async_copy(ws_hbm.at[l], w_ref.at[slot], sem.at[slot])

    def wsl(it, f, g):
        return pl.ds(it * WI + f * WF + g * WG, 128)

    def pro_layer(l, carry):
        slot = l % 2
        wcopy(l, slot).wait()

        @pl.when(l + 1 < L)
        def _():
            wcopy(l + 1, 1 - slot).start()
        w = w_ref.at[slot]
        xb = xf_ref[...].astype(BF16)
        toks = []
        KH = D // 2
        for n in range(D // 128):
            cols = pl.ds(n * 128, 128)
            y1 = jnp.dot(xb[:, :KH], w[pl.ds(0, KH), cols], preferred_element_type=F32)
            y2 = y1 + jnp.dot(xb[:, KH:], w[pl.ds(KH, KH), cols], preferred_element_type=F32)
            toks += [y1, y2]
            x0 = jnp.concatenate([xc_ref[pl.ds(0, HALF), cols], xl_ref[:, cols]], axis=0).astype(F32)
            b = bs_ref[l, :, cols].astype(F32)
            xf_ref[:, cols] = x0 * (y2 + b) + xf_ref[:, cols]

        def unpk(u):
            if pk != 1:
                return u.astype(F32)
            lo = pltpu.bitcast(u << 16, F32)
            hi = pltpu.bitcast(u & jnp.uint32(0xFFFF0000), F32)
            return jnp.concatenate([lo, hi], axis=0)

        def pack(x):
            if pk == 2:
                x4 = x.reshape(8, 2, 8, 128)
                y = jnp.concatenate([x4[:, 0], x4[:, 1]], axis=2).astype(BF16)
                return jnp.concatenate([y[:, :, :128], y[:, :, 128:]], axis=1).reshape(128, 128)
            if pk != 1:
                return x.astype(BF16)
            return pltpu.pack_elementwise([x[:64], x[64:]], packed_dtype=BF16)

        def w1(q, p, tok):
            v = []
            for Q in range(4):
                r, c = bits(Q, q, p)
                sc = -0.5 * LAM[Q] * LAM[q] * LAM[p]
                wb = w[pl.ds(r * 128, 128), pl.ds(c * 128, 128)]
                v.append(unpk(pltpu.bitcast(wb, U32) if pk == 1 else wb) * (anchored(sc, tok) if Q == 0 else sc))
            b11, s, t, b22 = v
            tr = b11 + b22
            for F, x in enumerate([tr, b11 - s, b11 + s, tr + (s + t), tr + tr]):
                buf[wsl(F, q, p)] = x

        def w2(F, p, tok):
            y = [buf[wsl(F, q, p)] for q in range(4)]
            y[0] = anchored(y[0], tok)
            for f, x in enumerate(a_tr(*y)):
                buf[wsl(5 + F, f, p)] = x

        def w3(I, i, tok):
            b11, s, t, b22 = [lin([(c * C, buf[wsl(5 + F, f, p)]) for C, F in BOP_OUT[I] for c, f in BOP[i]]) for p in range(4)]
            b11 = anchored(b11, tok)
            tr = b11 + b22
            trb = pack(tr)
            if fb:
                r = unpk(trb)
                e2 = (r - tr) * 0.5
                b11, b22, tr = b11 + e2, b22 + e2, r
            else:
                b22 = anchored(b22, tok)
            g = (tr + (s + t)) * 0.5
            out = {M1: trb, M2: b11 - s, M5: b22 + s, M6: b11 + s, M3: b22 - s, M7: g, M4: tr - g}
            for k, x in out.items():
                (t_ref if pk == 1 else tb)[tix(l, (I * 7 + i) * 7 + k)] = x if k == M1 else pack(x)

        st1 = [(cost(30, 8, 10), ('1', q, p)) for q in range(4) for p in range(4)]
        st2 = [(cost(14, 8, 8), ('2', F, p)) for F in range(5) for p in range(4)]
        st3 = []
        for I in range(7):
            for i in range(7):
                T = len(BOP_OUT[I]) * len(BOP[i])
                st3.append((cost(8 * (T - 1) + 27 + (10 if fb else 2), 8 * T, 7), ('3', I, i)))
        seq = []
        for t in range(8 + 2):
            cur = [[(c, key, t - si) for c, key in stg] for si, stg in enumerate([st1, st2, st3]) if 0 <= t - si < 8]
            m = max(len(x) for x in cur)
            merged = sorted((j / len(x), si, e) for si, x in enumerate(cur) for j, e in enumerate(x))
            seq += [e for _, _, e in merged]
        ntok = 64 * len(toks)
        fixed = np.zeros(len(toks))
        fixed[1::2] += cost(64 * 5, 64 * 3, 64)
        fixed[0::2] += cost(0, 0, 64)
        fixed[:2] += cost(128, 256, 128) * pw
        tot = sum(c for c, _, _ in seq)
        lv = water(fixed, np.ones(len(toks), bool), 0, len(toks), tot)
        cum = np.concatenate([[0], np.cumsum(np.maximum(lv - fixed, 0))])
        where = {}
        acc = 0.0
        for c, key, rp in seq:
            j = min(int(np.searchsorted(cum, acc, side='right')) - 1, len(toks) - 1)
            where[(key, rp)] = (j, min(int((acc - cum[j]) / (cum[j + 1] - cum[j]) * 64), 63))
            acc += c
        for stg, fn in ((st1, w1), (st2, w2), (st3, w3)):
            for _, key in stg:
                parts = []
                for rp in range(8):
                    j, r = where[(key, rp)]
                    tk = toks[j][8 * r:8 * r + 8]
                    parts += [tk] if pk == 1 else [tk, tk]
                fn(key[1], key[2], jnp.concatenate(parts * 2 if pk == 1 else parts, axis=0))
        return carry

    def prologue():
        wcopy(0, 0).start()
        for it in _z:
            buf[pl.ds(it * SI, SI)] = jnp.zeros((SI, 128), F32)
        colscale = jnp.concatenate([jnp.full((1, 128), SQ3 ** (-bin(c).count("1")), F32) for c in range(D // 128)], axis=1)
        beta = jnp.ones((1, D), F32)
        for l in range(L):
            beta = beta + bs_ref[l].astype(F32)
            for rp in range(4):
                bt_ref[l, rp] = jnp.broadcast_to(beta * colscale * SQ3 ** rp, (8, D))
        xf_ref[pl.ds(0, HALF), :] = xc_ref[pl.ds(0, HALF), :].astype(F32)
        xf_ref[pl.ds(HALF, HALF), :] = xl_ref[...].astype(F32)
        jax.lax.fori_loop(0, L, pro_layer, 0)
        sav_ref[...] = xf_ref[...].astype(BF16)
        regn = {}
        for Q in (1, 0):
            run_all(build('init', Q, L - 1, NG, regn, rel0=0))

    if only == 1:
        main_body()
        return
    if only == 2:
        prologue()
        o_ref[0:128, 0:tb.shape[-1]] = tb[z0, z0]
        return

    pl.when(step == 0)(prologue)
    pl.when(jnp.logical_and(step > 0, step < nsteps - 1))(main_body)

    @pl.when(step == 1)
    def _():
        o_ref[0:HALF, :] = sav_ref[0:HALF, :]

    @pl.when(step == nsteps - 1)
    def _():
        regp = {}
        for Q in (3, 2):
            run_all(build('final', Q, L - 1, -49, regp, dl_end=49))
        o_ref[HALF:, :] = sav_ref[HALF:, :]


@jax.jit
def pallas_standalone__dcn_v2_cross__recsys_kernel(x0, ws, bs):
    mo, lo, delay, w0, shift, ak, lat, slack, only, fb, afb, pw, pk = 5236471, 5762431, 4.0, 0.0, 2.0, 0, 0.4, 1.02, 0, 1, 0, 1.0, 3
    B, D = x0.shape
    L = ws.shape[0]
    tm = 2 * HALF
    nt = B // tm
    one = pl.Buffered(1)
    dig = lambda s: [int(c) - 1 for c in str(s)]
    return pl.pallas_call(
        functools.partial(_kernel, morder=dig(mo), lorder=dig(lo), shift=shift, ak=ak, delay=delay, w0=w0, lat=lat, slack=slack,
                          only=only, fb=fb, afb=afb, pw=pw, pk=pk),
        grid=(nt + 1,),
        in_specs=[
            pl.BlockSpec((tm, D), lambda i: (jnp.minimum(i, nt - 1), 0)),
            pl.BlockSpec((tm, D), lambda i: (jnp.maximum(i - 1, 0), 0)),
            pl.BlockSpec((HALF, D), lambda i: (2 * nt - 1, 0), pipeline_mode=one),
            pl.BlockSpec(memory_space=pl.ANY),
            pl.BlockSpec((L, 1, D), lambda i: (0, 0, 0), pipeline_mode=one),
        ],
        out_specs=pl.BlockSpec((tm, D), lambda i: (jnp.maximum(i - 1, 0), 0)),
        out_shape=jax.ShapeDtypeStruct((B, D), x0.dtype),
        scratch_shapes=[pltpu.SMEM((1,), jnp.int32), pltpu.VMEM((1, NI * SI, 128), F32), (pltpu.VMEM((L, 343, 128, 128), BF16) if pk == 3 else pltpu.VMEM((L, 172, 64, 256), U32)),
                        pltpu.VMEM((L, 4, 8, D), F32), pltpu.VMEM((2, D, D), BF16), pltpu.VMEM((tm, D), F32),
                        pltpu.VMEM((tm, D), BF16), pltpu.SemaphoreType.DMA((2,))],
        compiler_params=pltpu.CompilerParams(
            dimension_semantics=("arbitrary",),
            vmem_limit_bytes=127 * 1024 * 1024,
        ),
    )(x0, x0, x0, ws, bs.reshape(L, 1, D))
```

```python
import functools
import numpy as np
import jax
import jax.numpy as jnp
import jax.experimental.pallas as pl
import jax.experimental.pallas.tpu as pltpu

F32 = jnp.float32
BF16 = jnp.bfloat16
U32 = jnp.uint32
M1, M2, M3, M4, M5, M6, M7 = range(7)
SQ3 = float(np.sqrt(3.0))
LAM = [1.0, 1 / SQ3, SQ3, 1.0]
RL = 64
HALF = 4 * RL
AOP = {M1: [(1, 0)], M3: [(1, 1)], M4: [(1, 0), (-1, 1)], M5: [(1, 2)], M7: [(1, 0), (-1, 2)], M2: [(1, 3)], M6: [(1, 0), (-1, 3)]}
BOP = {M1: [(1, 0)], M2: [(1, 1)], M5: [(1, 0), (-1, 1)], M6: [(1, 2)], M3: [(1, 0), (-1, 2)], M7: [(1, 3)], M4: [(1, 0), (-1, 3)]}
BOP_OUT = {M1: [(1, 4)], M2: [(1, 1)], M5: [(1, 0), (-1, 1)], M6: [(1, 2)], M3: [(1, 0), (-1, 2)], M7: [(1, 3)], M4: [(1, 4), (-1, 3)]}
PRIMED = [M5, M2, M6]
FIN = {M1: (0, -1, [(1, M5), (1, M2), (1, M6)]), M4: (1, 1, [(-1, M2)]), M7: (2, 1, [(-1, M6)]), M3: (3, 1, [(-1, M5)])}

_n = [0]
def _it(k=1):
    r = list(range(_n[0], _n[0] + k)); _n[0] += k
    return r
GP, GM, TR, UP, UM = (_it()[0] for _ in range(5))
TMP = _it(2)
X0 = _it(4)
R3, R5 = _it() * 2, _it() * 2
HH, R4, R7, R2, R6 = (_it(2) for k in range(5))
DD, C22, ZZ = _it(3), _it(3), _it(3)
C11 = _it(2)
C11 = C11 + C11[1:]
NHEAD = _n[0]
YY = _it(4)
SS = _it(2)
NN, PP = _it(2)
NI = _n[0]
SG = RL + 8
SF = 4 * SG + 8
SI = 4 * SF + 8
WG = 128 + 8
WF = 4 * WG + 8
WI = 4 * WF + 8
assert 10 * WI <= NHEAD * SI


def lin(terms):
    k = next(i for i, t in enumerate(terms) if t[0] > 0)
    acc = terms[k][1]
    for i, (c, v) in enumerate(terms):
        if i != k:
            acc = acc + v if c > 0 else acc - v
    return acc


def a_tr(a11, s, t, a22):
    tr = a11 + a22
    return [tr, a11 - s, a11 + s, (tr + (s + t)) * 0.5]


def c_tr(e0, e1, e2, e3, half=0.5):
    h = e3 * half
    c22 = e0 + h
    return [(c22 + e1) + e2, h, (h + e1) - e2, c22]


class Item:
    def __init__(self, key, cost, rel, dl, preds, fn):
        self.key, self.cost, self.rel, self.dl, self.preds, self.fn, self.pos = key, cost, rel, dl, preds, fn, None


def water(fixed, free, a, b, work):
    f = np.sort(fixed[a:b][free[a:b]])
    if len(f) == 0:
        return np.inf
    lv = (work + np.cumsum(f)) / np.arange(1, len(f) + 1)
    return lv[np.nonzero(lv >= f)[0][-1]]


def place(items, fixedv, lat, slack, cap, decay):
    fixed = fixedv.sum(1)
    n = len(fixed)
    jobs = {}
    for it in items:
        it.dl = int(np.floor(it.dl))
        k = (int(np.ceil(it.rel)), it.dl)
        jobs[k] = jobs.get(k, 0.0) + it.cost.sum()
    free = np.ones(n, bool)
    room = np.zeros(n)
    while jobs:
        best = None
        for a in sorted({k[0] for k in jobs}):
            for b in sorted({k[1] for k in jobs}):
                w = sum(v for k, v in jobs.items() if k[0] >= a and k[1] <= b)
                if b > a and w > 0:
                    lv = water(fixed, free, a, b, w)
                    if best is None or lv > best[0]:
                        best = (lv, a, b)
        lv, a, b = best
        idx = np.arange(a, b)[free[a:b]]
        room[idx] = np.maximum(lv - fixed[idx], 0)
        free[a:b] = False
        jobs = {k: v for k, v in jobs.items() if not (k[0] >= a and k[1] <= b)}
    room = room * slack
    rcum = np.concatenate([[0], np.cumsum(room)])
    dls = np.array(sorted({it.dl for it in items}))
    due = np.array([sum(it.cost.sum() for it in items if it.dl == d) for d in dls])
    streams = {}
    for it in items:
        streams.setdefault((it.dl, it.kind) + it.key[:3], []).append(it)
    keys = sorted(streams)
    debt = 0.0
    hist = np.zeros(3)
    for g in range(n):
        used = debt
        r = room[g]
        cur = fixedv[g] + hist
        while keys and (used < r or keys[0][0] <= g + 1):
            t = g + min(used / max(r, 1e-9), 0.99)
            lax_ = np.minimum.accumulate(np.where(dls > g, rcum[np.minimum(dls, n)] - rcum[g] - used - np.cumsum(due), np.inf))
            cands = []
            for key in keys:
                for it in streams[key][:8]:
                    if it.rel <= t and all(p.pos is not None and (p.pos + lat <= t or used >= r) for p in it.preds):
                        cands.append(it)
                        break
            if not cands:
                assert used < r
                used += r / 16
                continue
            ok = []
            for it in cands:
                j = int(np.searchsorted(dls, it.dl))
                if it.dl == cands[0].dl or j == 0 or lax_[j - 1] >= it.cost.sum():
                    ok.append(it)
            score = lambda it: np.max((cur + it.cost) / (cur + it.cost).sum())
            it = min(ok, key=score)
            if np.max(cur - hist + it.cost) > cap and lax_[-1] >= r - used and used < r:
                break
            key = (it.dl, it.kind) + it.key[:3]
            streams[key].remove(it)
            if not streams[key]:
                keys.remove(key)
            due[int(np.searchsorted(dls, it.dl))] -= it.cost.sum()
            it.pos = t
            used += it.cost.sum()
            cur = cur + it.cost
        debt = max(used - r, 0.0)
        hist = cur * decay
    assert not keys


def _kernel(x_hbm, ws_hbm, bs_hbm, o_hbm, z_ref, buf_ref, t_ref, bt_ref, bp_ref, w_ref, xf_ref, xin_ref, ost_ref, bs_ref, sem, *,
            morder, lorder0, shift, ak, delay, w0, lat, slack, only, fb, afb, pw, dstart, dwait, off, endm, wst, gm, wfirst, pro, sfb, cap, decay):
    L = bs_ref.shape[0]
    B, D = x_hbm.shape
    TM = 2 * HALF
    nt = B // TM
    tu = t_ref.bitcast(U32)
    env = {}

    def enter(i):
        env['z'] = z_ref[0]
        env['buf'] = buf_ref.at[env['z']]
        env['xc'] = xin_ref.at[i & 3]
        env['xp'] = xin_ref.at[(i + 3) & 3]
        env['o'] = ost_ref.at[i & 1]

    class View:
        def __init__(self, name):
            self.name = name
        def __getitem__(self, idx):
            return env[self.name][idx]
        def __setitem__(self, idx, v):
            env[self.name][idx] = v
    buf, xc_ref, xp_ref, o_ref = View('buf'), View('xc'), View('xp'), View('o')

    def anchored(v, tok):
        if tok is None:
            return v
        return jnp.where(jnp.full(tok.shape, env['z'], jnp.int32) == 0, v, tok)

    def sl(it, f, g):
        return pl.ds(it * SI + f * SF + g * SG, RL)

    def bits(Q, q, p):
        return (Q // 2) * 4 + (q // 2) * 2 + p // 2, (Q % 2) * 4 + (q % 2) * 2 + p % 2

    def io_idx(Q, q, p):
        r, c = bits(Q, q, p)
        return pl.ds((r ^ 4) * RL, RL), pl.ds(c * 128, 128)

    def use_sfb(it, f):
        return sfb == 28 or (sfb >= 7 and f == 0) or (sfb >= 10 and it == TR)

    def put_f(Q, f, v, par):
        ld = lambda it: [buf[sl(it, f, g)] for g in range(4)]
        add = lambda x, y: [a + b for a, b in zip(x, y)]
        sub = lambda x, y: [a - b for a, b in zip(x, y)]
        if Q == 1:
            out = {SS[par]: v}
        elif Q == 0:
            s = ld(SS[par])
            out = {NN: sub(v, s), PP: add(v, s)}
        elif Q == 3:
            s = ld(SS[par])
            up = add(v, s)
            out = {TR: add(up, ld(NN)), UP: up, UM: sub(v, s)}
        else:
            w = add(v, ld(SS[par]))
            tr = ld(TR)
            out = {GP: add(tr, w), GM: sub(tr, w)}
        for it, x in out.items():
            if Q != 1 and use_sfb(it, f):
                r = x[0].astype(BF16).astype(F32)
                e2 = (r - x[0]) * 0.5
                x = [r] + [y + e2 for y in x[1:]]
            for g in range(4):
                buf[sl(it, f, g)] = x[g]

    def lcost(Q, f):
        v, ld, st = {0: (15, 8, 8), 1: (7, 4, 4), 2: (19, 12, 8), 3: (19, 12, 12)}[Q]
        v += 7 * sum(use_sfb(it, f) for it in {0: [NN, PP], 1: [], 2: [GP, GM], 3: [TR, UP, UM]}[Q])
        return cost(v, ld, st)

    def put_y(Q, p, y):
        for f in range(4):
            buf[sl(YY[Q], f, p)] = y[f]

    def pass_init(Q, p, tok):
        xs = []
        for q in range(4):
            lam = LAM[Q] * LAM[q] * LAM[p]
            v = xc_ref[io_idx(Q, q, p)].astype(F32)
            if Q >= 2 or q == 0:
                v = anchored(v, tok)
            if Q >= 2:
                buf[sl(X0[Q], q, p)] = v
            xs.append(v if abs(lam - 1) < 1e-9 else v * lam)
        put_y(Q, p, a_tr(*xs))

    KT = {1: ([(1, R3), (-1, R5)], DD), 0: ([(1, HH), (1, R4), (1, R7)], C11), 3: ([(1, HH), (1, R2), (1, R6)], C22),
          2: ([(1, R4), (-1, R7), (-1, R2), (1, R6)], ZZ)}

    def pass_k(Q, f, l, tok):
        par = l % 2
        terms, dst = KT[Q]
        e = [lin([(c, buf[sl(it[par], f, g)]) for c, it in terms]) for g in range(4)]
        c = c_tr(*e, half=anchored(0.5, tok))
        for p in range(4):
            v = c[p] if l == 0 else c[p] + buf[sl(dst[1 - par], f, p)]
            buf[sl(dst[2 if l == L - 1 else par], f, p)] = v

    def mix_x(Q, p, l, tok):
        par = 2 if l == L - 1 else l % 2
        if Q == 2:
            e = [buf[sl(DD[par], f, p)] + buf[sl(ZZ[par], f, p)] for f in range(4)]
        else:
            e = [buf[sl(KT[Q][1][par], f, p)] for f in range(4)]
        c = c_tr(*e, half=anchored(0.5, tok))
        res = []
        for q in range(4):
            if (Q < 2 and l == 0) or (Q >= 2 and l == L - 1):
                x0 = xp_ref[io_idx(Q, q, p)].astype(F32)
                if Q < 2:
                    x0 = anchored(x0, tok)
                    buf[sl(X0[Q], q, p)] = x0
            else:
                x0 = buf[sl(X0[Q], q, p)]
            r, cb = bits(Q, q, p)
            b = bt_ref[l, bin(r).count("1"), :, pl.ds(cb * 128, 128)]
            res.append((c[q] + jnp.concatenate([b] * (RL // 8), axis=0)) * x0)
        return res

    def pass_m(Q, p, l, tok):
        put_y(Q, p, a_tr(*mix_x(Q, p, l, tok)))

    def pass_l(Q, f, par, tok):
        y = [buf[sl(YY[Q], f, p)] for p in range(4)]
        y[0] = anchored(y[0], tok)
        put_f(Q, f, a_tr(*y), par)

    def pass_final(Q, p, l, tok):
        xt = mix_x(Q, p, l, tok)
        for q in range(4):
            lam = LAM[Q] * LAM[q] * LAM[p]
            v = xt[q] if abs(lam - 1) < 1e-9 else xt[q] * (1 / lam)
            o_ref[io_idx(Q, q, p)] = v.astype(BF16)

    def use_afb(I, i):
        return afb == 2 or (afb == 1 and (I == M1 or i == M1))

    LOA = {1: ['4276351', '3514276', '3542761', '1427635'], 2: ['3542761', '7613542', '7635421', '1354276'],
           3: ['3576421', '4213576', '4235761', '1357642'], 4: ['4276351', '3514276', '4276351', '1427635'],
           5: ['6275431', '4316275', '4362751', '1627543']}

    def lorder_of(G):
        if len(lorder0) == 7:
            return lorder0
        return [int(c) - 1 for c in LOA[lorder0[0] + 1][(7 * G + off) % 4]]

    def group(l, ph, I, src, acc, dst, i):
        lorder = lorder_of(l * 49 + ph * 7 + morder.index(i))
        tmp = TMP[(l * 7 + ph) % 2]
        fs = [lin([(c, buf[sl(src, f, g)]) for c, f in AOP[i]]) for g in range(4)]
        ops = {}
        if use_afb(I, i):
            ops[M1] = fs[0].astype(BF16)
            r = ops[M1].astype(F32)
            e2 = (r - fs[0]) * 0.5
            fs = [r] + [v + e2 for v in fs[1:]]
        n = {}
        for k in lorder:
            op = ops[k] if k in ops else lin([(c, fs[g]) for c, g in AOP[k]]).astype(BF16)
            w = pltpu.bitcast(tu[l, (I * 7 + i) * 7 + k], BF16)
            n[k] = jnp.dot(op, w, preferred_element_type=F32)
        e = [None] * 4
        for k, (f, sg, rt) in FIN.items():
            terms = dict([(k, sg)] + [(x, c) for c, x in rt])
            e[f] = lin([(terms[j], n[j]) for j in lorder if j in terms])
        if i in PRIMED:
            for g in range(4):
                buf[sl(tmp, PRIMED.index(i), g)] = e[g]
        else:
            f, sg, rt = FIN[i]
            so = -1 if I == M1 else 1
            for g in range(4):
                terms = [(so * sg, e[g])] + [(so * c, buf[sl(tmp, PRIMED.index(k), g)]) for c, k in rt] + [(1, buf[sl(it, f, g)]) for it in acc]
                if terms[0][0] < 0:
                    j = next(j for j, t in enumerate(terms) if t[0] > 0)
                    terms = [terms[j], terms[0]] + [t for jj, t in enumerate(terms) if jj not in (0, j)]
                buf[sl(dst, f, g)] = lin(terms)
        return [n[k] for k in lorder]

    P = functools.partial
    cost = lambda valu, ld, st: np.array([valu / 4, ld / 3, st * wst])

    def phases(l):
        par = l % 2
        return [(M3, NN, [], R3[par]), (M5, PP, [], R5[par]), (M1, TR, [R3[par], R5[par]], HH[par]), (M4, UP, [], R4[par]),
                (M7, UM, [], R7[par]), (M2, GP, [], R2[par]), (M6, GM, [], R6[par])]

    NS = (343 * L + off + 3) // 4
    slot_of = lambda G, k: (7 * G + k + off) // 4

    def fixed_costs():
        ca, cc = np.zeros((NS + 8, 3)), np.zeros((NS + 8, 3))
        G = 0
        for l in range(L):
            for I, src, acc, dst in phases(l):
                for i in morder:
                    T = len(AOP[i])
                    lorder = lorder_of(G)
                    kpos = {k: j for j, k in enumerate(lorder)}
                    seen = set()
                    x = 8 if use_afb(I, i) else 0
                    for j, k in enumerate(lorder):
                        new = ({g for _, g in AOP[k]} | ({0} if x else set())) - seen
                        seen |= new
                        ca[slot_of(G, j)] += cost(4 + 8 * (len(AOP[k]) - 1) + (8 * (T - 1) + x) * len(new) + (2 * x if 0 in new else 0), 8 + 8 * T * len(new), 0)
                    nr = 0 if i in PRIMED else len(FIN[i][2]) + len(acc)
                    for k, (f, sg, rt) in FIN.items():
                        arr = sorted([kpos[k]] + [kpos[x] for _, x in rt])
                        for j in arr[1:]:
                            cc[slot_of(G, j)] += cost(8, 0, 0)
                        cc[slot_of(G, arr[-1])] += cost(8 * nr, 8 * nr, 8)
                    G += 1
        lo = int(np.floor(shift)); fr = shift - lo
        return cc[:NS] + (1 - fr) * ca[lo:lo + NS] + fr * ca[lo + 1:lo + NS + 1]

    NG = 49 * L
    t_end = lambda G: slot_of(G, 6) + 1
    t_beg = lambda G: min(slot_of(G, 0), NS)
    done_at = {f: morder.index(i) for i, (f, _, _) in FIN.items()}
    PH_DONE = {1: 1, 0: 4, 3: 6, 2: 6}
    PH_USE = {1: 7, 0: 7, 3: 9, 2: 12}

    def build(kind, Q, l, base, reg, rel0=None, dl_end=None):
        io = Q < 2 and l == 0
        rel = [t_end(base + PH_DONE[Q] * 7 + done_at[f]) + w0 for f in range(4)]
        if kind == 'init':
            rel = [rel0] * 4
        dl = dl_end if kind == 'final' else min(slot_of(base + PH_USE[Q] * 7, 0) - delay, NS)
        x = 4 if Q == 2 else 0
        stages = []
        if kind != 'init':
            nt = len(KT[Q][0])
            stages.append(('K', cost(4 * nt + 7, 4 * nt + 4, 4), [P(pass_k, Q, f, l) for f in range(4)]))
        if kind == 'init':
            stages.append(('M', cost(18 if Q >= 2 else 15, 4, 8 if Q >= 2 else 4), [P(pass_init, Q, p) for p in range(4)]))
        elif kind == 'mix':
            stages.append(('M', cost(21 + x + (8 if io else 0), 12 + x, 8 if io else 4), [P(pass_m, Q, p, l) for p in range(4)]))
        else:
            stages.append(('M', cost(22 + x + (4 if Q >= 2 else 0), 12 + x, 4), [P(pass_final, Q, p, l) for p in range(4)]))
        if kind != 'final':
            stages.append(('L', None, [P(pass_l, Q, f, (l + 1) % 2) for f in range(4)]))
        items = []
        for t in range(8 + len(stages) - 1):
            for j in range(4):
                for si, (nm, c, fns) in enumerate(stages):
                    r = t - si
                    if not 0 <= r < 8:
                        continue
                    pre = [reg[(stages[si - 1][0], Q, l, jj, r)] for jj in range(4)] if si else []
                    if nm == 'M' and Q == 2:
                        pre += [reg[kk] for kk in [('K', 1, l, f, r) for f in range(4)] if kk in reg]
                    if nm == 'L':
                        pre += [reg[('L', d, l, j, r)] for d in {0: [1], 1: [], 3: [1, 0], 2: [1, 3]}[Q] if ('L', d, l, j, r) in reg]
                    it = Item((nm, Q, l, j, r), lcost(Q, j) if nm == 'L' else c, max(rel[j] if nm == 'K' else max(rel), 0), dl, pre, fns[j])
                    it.kind = kind
                    reg[it.key] = it
                    items.append(it)
        return items

    def run_all(items):
        for nm in 'KML':
            for it in items:
                if it.key[0] == nm and it.key[4] == 0:
                    it.fn(None)

    def rows(r, n):
        return pl.ds(pl.multiple_of(r, HALF), n)

    def fetch_copy(i):
        nxt = jnp.minimum(i + 1, nt - 1)
        return pltpu.make_async_copy(x_hbm.at[rows(nxt * TM, TM)], xin_ref.at[(i + 1) & 3], sem.at[2])

    def top_copy(i):
        return pltpu.make_async_copy(ost_ref.at[jnp.where(i == 1, 2, (i + 1) & 1), pl.ds(HALF, HALF)],
                                     o_hbm.at[rows(jnp.where(i == 1, B - HALF, (i - 2) * TM + HALF), HALF)], sem.at[4])

    def bot_copy(i):
        return pltpu.make_async_copy(ost_ref.at[jnp.where(i == 1, 2, i & 1), pl.ds(0, HALF)],
                                     o_hbm.at[rows((i - 1) * TM, HALF)], sem.at[3])

    def main_body(step, carry):
        enter(step)
        copies = [fetch_copy(step), top_copy(step), bot_copy(step)]
        copies[0].start()
        copies[1].start()
        reg, regp, regn = {}, {}, {}
        items = []
        for Q in (3, 2):
            items += build('init', Q, -1, -49, reg, rel0=0)
        for Q in (3, 2):
            items += build('final', Q, L - 1, -49, regp, dl_end=t_beg(49))
        for it in regp.values():
            if it.key[0] == 'M':
                it.dl = t_beg(49 * (L - 1))
        for l in range(L):
            for Q in (1, 0, 3, 2):
                if l < L - 1:
                    items += build('mix', Q, l, 49 * l, reg)
                elif Q < 2:
                    items += build('final', Q, l, 49 * l, reg, dl_end=NS)
        for Q in (1, 0):
            items += build('init', Q, L - 1, NG, regn, rel0=t_beg(49 * (L - 1)))
        for it in regn.values():
            if it.key[0] == 'L' and it.key[1] == 0:
                it.rel = t_beg(49 * (L - 1) + 14)
        for it in items:
            it.dl = min(it.dl, NS - endm)
        place(items, fixed_costs(), lat, slack, cap, decay)
        batches = {}
        for it in items:
            batches.setdefault(id(it.fn), []).append(it)
            it.prod = max(min(4 * int(it.pos) + ak - off, 343 * L - 1), 0)
            it.row = min(int((it.pos - int(it.pos)) * 8), 7)
        blist = sorted(batches.values(), key=lambda b: (max(it.pos for it in b), 'KML'.index(b[0].key[0])))
        toks = []
        k = 0
        for l in range(L):
            for ph, (I, src, acc, dst) in enumerate(phases(l)):
                for i in morder:
                    if len(toks) == 343 * (L - 1) + 7 * dstart:
                        assert all(bb[0].kind != 'final' or bb[0].key[1] < 2 for bb in blist[k:])
                        copies[2].start()
                    toks += group(l, ph, I, src, acc, dst, i)
                    while k < len(blist) and max(it.prod for it in blist[k]) < len(toks):
                        b = sorted(blist[k], key=lambda it: it.key[4])
                        b[0].fn(jnp.concatenate([toks[it.prod][8 * it.row:8 * it.row + 8] for it in b], axis=0))
                        k += 1
        assert k == len(blist)
        for c in copies:
            c.wait()
        return carry

    def wcopy(l, slot):
        return pltpu.make_async_copy(ws_hbm.at[l], w_ref.at[slot], sem.at[slot])

    def second():
        return pltpu.make_async_copy(x_hbm.at[pl.ds(TM, TM)], xin_ref.at[1], sem.at[2])

    def wsl(it, f, g):
        return pl.ds(it * WI + f * WF + g * WG, 128)

    def pro_layer(l, carry):
        enter(0)
        slot = l & 1
        wcopy(l, slot).wait()

        @pl.when(l + 1 < L)
        def _():
            wcopy(l + 1, 1 - slot).start()

        @pl.when(l + 1 == L)
        def _():
            second().start()
        w = w_ref.at[slot]
        xb = xf_ref[0].astype(BF16)
        toks = []
        KH = D // 2
        for n in range(D // 128):
            cols = pl.ds(n * 128, 128)
            y1 = jnp.dot(xb[:, :KH], w[pl.ds(0, KH), cols], preferred_element_type=F32)
            y2 = y1 + jnp.dot(xb[:, KH:], w[pl.ds(KH, KH), cols], preferred_element_type=F32)
            toks += [y1, y2]
            x0 = xf_ref[1, :, cols] if pro else xp_ref[:, cols].astype(F32)
            b = bp_ref[l, pl.ds(0, 1), cols]
            xf_ref[0, :, cols] = x0 * (y2 + b) + xf_ref[0, :, cols]

        def w1(q, p, tok):
            v = []
            for Q in range(4):
                r, c = bits(Q, q, p)
                sc = -0.5 * LAM[Q] * LAM[q] * LAM[p]
                wb = w[pl.ds(r * 128, 128), pl.ds(c * 128, 128)]
                v.append(wb.astype(F32) * (anchored(sc, tok) if Q == 0 else sc))
            b11, s, t, b22 = v
            tr = b11 + b22
            for F, x in enumerate([tr, b11 - s, b11 + s, tr + (s + t), tr + tr]):
                buf[wsl(F, q, p)] = x

        def w2(F, p, tok):
            y = [buf[wsl(F, q, p)] for q in range(4)]
            y[0] = anchored(y[0], tok)
            for f, x in enumerate(a_tr(*y)):
                buf[wsl(5 + F, f, p)] = x

        def w3(I, i, tok):
            b11, s, t, b22 = [lin([(c * C, buf[wsl(5 + F, f, p)]) for C, F in BOP_OUT[I] for c, f in BOP[i]]) for p in range(4)]
            half = 0.5
            if pro >= 2:
                half = anchored(0.5, tok)
            else:
                b11 = anchored(b11, tok)
            tr = b11 + b22
            trb = tr.astype(BF16)
            if fb:
                r = trb.astype(F32)
                e2 = (r - tr) * half
                b11, b22, tr = b11 + e2, b22 + e2, r
            else:
                b22 = anchored(b22, tok)
            g = (tr + (s + t)) * half
            out = {M1: trb, M2: b11 - s, M5: b22 + s, M6: b11 + s, M3: b22 - s, M7: g, M4: tr - g}
            for k, x in out.items():
                t_ref[l, (I * 7 + i) * 7 + k] = x.astype(BF16)

        cost = lambda valu, ld, st: valu / 4 + ld / 3 + st
        st1 = [(cost(30, 8, 10), ('1', q, p)) for q in range(4) for p in range(4)]
        st2 = [(cost(14, 8, 8), ('2', F, p)) for F in range(5) for p in range(4)]
        st3 = []
        for I in range(7):
            for i in range(7):
                T = len(BOP_OUT[I]) * len(BOP[i])
                st3.append((cost(8 * (T - 1) + 27 + (10 if fb else 2), 8 * T, 7), ('3', I, i)))
        seq = []
        for t in range(8 + 2):
            cur = [[(c, key, t - si) for c, key in stg] for si, stg in enumerate([st1, st2, st3]) if 0 <= t - si < 8]
            m = max(len(x) for x in cur)
            merged = sorted((j / len(x), si, e) for si, x in enumerate(cur) for j, e in enumerate(x))
            seq += [e for _, _, e in merged]
        ntok = 64 * len(toks)
        fixed = np.zeros(len(toks))
        fixed[1::2] += cost(64 * 5, 64 * 3, 64)
        fixed[0::2] += cost(0, 0, 64)
        fixed[:2] += cost(128, 256, 128) * pw
        tot = sum(c for c, _, _ in seq)
        lv = water(fixed, np.ones(len(toks), bool), 0, len(toks), tot)
        cum = np.concatenate([[0], np.cumsum(np.maximum(lv - fixed, 0))])
        where = {}
        acc = 0.0
        for c, key, rp in seq:
            j = min(int(np.searchsorted(cum, acc, side='right')) - 1, len(toks) - 1)
            where[(key, rp)] = (j, min(int((acc - cum[j]) / (cum[j + 1] - cum[j]) * 64), 63))
            acc += c
        for stg, fn in ((st1, w1), (st2, w2), (st3, w3)):
            for _, key in stg:
                parts = []
                for rp in range(8):
                    j, r = where[(key, rp)]
                    tk = toks[j][8 * r:8 * r + 8]
                    parts += [tk, tk]
                fn(key[1], key[2], jnp.concatenate(parts, axis=0))
        return carry

    def prologue():
        z_ref[0] = 0
        first = [pltpu.make_async_copy(x_hbm.at[pl.ds(0, HALF)], xin_ref.at[3, pl.ds(0, HALF)], sem.at[2]),
                 pltpu.make_async_copy(x_hbm.at[pl.ds(B - HALF, HALF)], xin_ref.at[3, pl.ds(HALF, HALF)], sem.at[3]),
                 pltpu.make_async_copy(x_hbm.at[pl.ds(HALF, HALF)], xin_ref.at[0, pl.ds(HALF, HALF)], sem.at[4])]
        bcopy = pltpu.make_async_copy(bs_hbm, bs_ref, sem.at[1])
        bcopy.start()
        if wfirst == 1:
            wcopy(0, 0).start()
        for c in first:
            c.start()
        if wfirst == 0:
            wcopy(0, 0).start()
        if wfirst >= 2:
            r = D // wfirst
            for k in range(wfirst):
                pltpu.make_async_copy(ws_hbm.at[0, pl.ds(k * r, r)], w_ref.at[0, pl.ds(k * r, r)], sem.at[0]).start()
        bcopy.wait()
        colscale = jnp.concatenate([jnp.full((1, 128), SQ3 ** (-bin(c).count("1")), F32) for c in range(D // 128)], axis=1)
        beta = jnp.ones((1, D), F32)
        for l in range(L):
            bl = bs_ref[l:l + 1, :].astype(F32)
            bp_ref[l] = jnp.broadcast_to(bl, (8, D))
            beta = beta + bl
            for rp in range(4):
                bt_ref[l, rp] = jnp.broadcast_to(beta * colscale * SQ3 ** rp, (8, D))
        for c in first:
            c.wait()
        enter(0)
        xf_ref[0] = xp_ref[...].astype(F32)
        if pro:
            xf_ref[1] = xp_ref[...].astype(F32)
        regn = {}
        for Q in (1, 0):
            run_all(build('init', Q, L - 1, NG, regn, rel0=0))
        jax.lax.fori_loop(0, L, pro_layer, 0)
        ost_ref[2] = xf_ref[0].astype(BF16)
        second().wait()

    def drain():
        enter(nt)
        copies = [top_copy(jnp.int32(nt))]
        copies[0].start()
        for Q in (3, 2):
            for f in range(4):
                pass_k(Q, f, L - 1, None)
        for h in range(2):
            for Q in (3, 2):
                for p in (2 * h, 2 * h + 1):
                    pass_final(Q, p, L - 1, None)
            for j in range(2):
                r = (2 * j + h) * RL
                copies.append(pltpu.make_async_copy(ost_ref.at[nt % 2, pl.ds(r, RL)], o_hbm.at[pl.ds(B - TM + r, RL)], sem.at[2 * h + j]))
                copies[-1].start()
        for c in copies:
            c.wait()

    if gm:
        step = pl.program_id(0)
        pl.when(step == 0)(prologue)
        @pl.when(step > 0)
        def _():
            main_body(step, 0)
        pl.when(step == nt - 1)(drain)
        return
    if only != 1:
        prologue()
    if only == 2:
        ost_ref[0, 0:128, 0:128] = t_ref[z_ref[0], z_ref[0]]
    else:
        jax.lax.fori_loop(1, nt, main_body, 0)
    if only != 1:
        drain()


def _call(x0, ws, bs, nl=6, mo=2563471, lo=6275431, delay=4.0, w0=0.5, shift=2.0, ak=1, lat=0.25, slack=1.02, only=0, fb=1, afb=0, pw=1.0,
           dstart=3, dwait=999, nbc=1, off=2, endm=1, wst=1.0, gm=0, wfirst=0, pro=0, sfb=10, cap=50, decay=0.25):
    if nl != 6:
        ws = ws[:nl]; bs = bs[:nl]
    B, D = x0.shape
    L = ws.shape[0]
    tm = 2 * HALF
    dig = lambda s: [int(c) - 1 for c in str(s)]
    return pl.pallas_call(
        functools.partial(_kernel, morder=dig(mo), lorder0=dig(lo), shift=shift, ak=ak, delay=delay, w0=w0, lat=lat, slack=slack,
                          only=only, fb=fb, afb=afb, pw=pw, dstart=dstart, dwait=dwait, off=off, endm=endm, wst=wst, gm=gm, wfirst=wfirst, pro=pro, sfb=sfb, cap=cap, decay=decay),
        grid=(B // tm,) if gm else (),
        in_specs=[
            pl.BlockSpec(memory_space=pl.ANY),
            pl.BlockSpec(memory_space=pl.ANY),
            pl.BlockSpec(memory_space=pl.ANY),
        ],
        out_specs=pl.BlockSpec(memory_space=pl.ANY),
        out_shape=jax.ShapeDtypeStruct((B, D), x0.dtype),
        scratch_shapes=[pltpu.SMEM((1,), jnp.int32), pltpu.VMEM((1, -(-NI * SI // 32) * 32, 128), F32), pltpu.VMEM((L, 343, 128, 128), BF16),
                        pltpu.VMEM((L, 4, 8, D), F32), pltpu.VMEM((L, 8, D), F32), pltpu.VMEM((2, D, D), BF16),
                        pltpu.VMEM((2, tm, D), F32), pltpu.VMEM((4, tm, D), BF16), pltpu.VMEM((3, tm, D), BF16), pltpu.VMEM((L, D), BF16),
                        pltpu.SemaphoreType.DMA((5,))],
        compiler_params=pltpu.CompilerParams(
            vmem_limit_bytes=127 * 1024 * 1024,
            disable_bounds_checks=bool(nbc),
        ),
    )(x0, ws, bs)


@jax.jit
def pallas_standalone__dcn_v2_cross__recsys_kernel(x0, ws, bs):
    return _call(x0, ws, bs)
```

```python
import functools

import numpy as np
import jax
import jax.numpy as jnp
from jax import lax
import jax.experimental.pallas as pl
import jax.experimental.pallas.tpu as pltpu

F32 = jnp.float32
BF16 = jnp.bfloat16
U32 = jnp.uint32

M1, M2, M3, M4, M5, M6, M7 = range(7)
SQ3 = float(np.sqrt(3.0))
LAM = (1.0, 1 / SQ3, SQ3, 1.0)
RL = 64
HALF = 4 * RL
TM = 2 * HALF
AOP = {M1: [(1, 0)], M3: [(1, 1)], M4: [(1, 0), (-1, 1)], M5: [(1, 2)], M7: [(1, 0), (-1, 2)],
       M2: [(1, 3)], M6: [(1, 0), (-1, 3)]}
BOP = {M1: [(1, 0)], M2: [(1, 1)], M5: [(1, 0), (-1, 1)], M6: [(1, 2)], M3: [(1, 0), (-1, 2)],
       M7: [(1, 3)], M4: [(1, 0), (-1, 3)]}
BOP_OUT = {**BOP, M1: [(1, 4)], M4: [(1, 4), (-1, 3)]}
PRIMED = [M5, M2, M6]
FIN = {M1: (0, -1, [(1, M5), (1, M2), (1, M6)]), M4: (1, 1, [(-1, M2)]), M7: (2, 1, [(-1, M6)]),
       M3: (3, 1, [(-1, M5)])}

GP, GM, TR, UP, UM = range(5)
TMP = [5, 6]
X0 = [7, 8, 9, 10]
R3, R5 = [11, 11], [12, 12]
HH, R4, R7, R2, R6 = [13, 14], [15, 16], [17, 18], [19, 20], [21, 22]
DD, C22, ZZ, C11 = [23, 24, 25], [26, 27, 28], [29, 30, 31], [32, 33, 33]
YY = [34, 35, 36, 37]
SS = [38, 39]
NN, PP = 40, 41
NI = 44
KT = {1: ([(1, R3), (-1, R5)], DD), 0: ([(1, HH), (1, R4), (1, R7)], C11),
      3: ([(1, HH), (1, R2), (1, R6)], C22), 2: ([(1, R4), (-1, R7), (-1, R2), (1, R6)], ZZ)}
PH_DONE = {1: 1, 0: 4, 3: 6, 2: 6}
PH_USE = {1: 7, 0: 7, 3: 9, 2: 12}

CFG = dict(mo=6254371, lo='6275341x6275431x2675431x1576243', delay=2.5, w0=0.0, shift=2.25, ak=0, lat=0.15, slack=1.02,
           endm=0, wst=1.2, cap=50, decay=0, po=13, lead=3, leadk=3, pace=0.45)


def lin(terms):
    k = next(i for i, t in enumerate(terms) if t[0] > 0)
    acc = terms[k][1]
    for i, (c, v) in enumerate(terms):
        if i != k:
            acc = acc + v if c > 0 else acc - v
    return acc


def a_tr(a11, s, t, a22):
    tr = a11 + a22
    return [tr, a11 - s, a11 + s, (tr + (s + t)) * 0.5]


def c_tr(e0, e1, e2, e3, half):
    h = e3 * half
    c22 = e0 + h
    return [(c22 + e1) + e2, h, (h + e1) - e2, c22]


def bits(Q, q, p):
    return (Q // 2) * 4 + (q // 2) * 2 + p // 2, (Q % 2) * 4 + (q % 2) * 2 + p % 2


def stack(xs):
    return jnp.concatenate(xs, axis=0).reshape((len(xs),) + xs[0].shape)


class Item:
    def __init__(self, stage, j, r, cost, rel, dl, preds):
        self.stage, self.j, self.r, self.cost, self.rel, self.dl, self.preds = stage, j, r, cost, rel, dl, preds
        self.pos = None


def water(fixed, work):
    f = np.sort(fixed)
    if len(f) == 0:
        return np.inf
    lv = (work + np.cumsum(f)) / np.arange(1, len(f) + 1)
    return lv[np.nonzero(lv >= f)[0][-1]]


def place(items, fixedv, cfg):
    fixed = fixedv.sum(1)
    n = len(fixed)
    jobs = {}
    for it in items:
        it.dl = int(np.floor(it.dl))
        k = (int(np.ceil(it.rel)), it.dl)
        jobs[k] = jobs.get(k, 0.0) + it.cost.sum()
    free = np.ones(n, bool)
    room = np.zeros(n)
    while jobs:
        best = None
        for a in sorted({k[0] for k in jobs}):
            for b in sorted({k[1] for k in jobs}):
                w = sum(v for k, v in jobs.items() if k[0] >= a and k[1] <= b)
                if b > a and w > 0:
                    lv = water(fixed[a:b][free[a:b]], w)
                    if best is None or lv > best[0]:
                        best = (lv, a, b)
        lv, a, b = best
        idx = np.arange(a, b)[free[a:b]]
        room[idx] = np.maximum(lv - fixed[idx], 0)
        free[a:b] = False
        jobs = {k: v for k, v in jobs.items() if not (k[0] >= a and k[1] <= b)}
    room = room * cfg['slack']
    rcum = np.concatenate([[0], np.cumsum(room)])
    dls = np.array(sorted({it.dl for it in items}))
    due = np.array([sum(it.cost.sum() for it in items if it.dl == d) for d in dls])
    streams = {}
    for it in items:
        streams.setdefault((it.dl,) + it.stage, []).append(it)
    keys = sorted(streams)
    debt = 0.0
    hist = np.zeros(3)
    for g in range(n):
        used = debt
        r = room[g]
        cur = fixedv[g] + hist
        while keys and (used < r or keys[0][0] <= g + 1):
            t = g + min(used / max(r, 1e-9), 0.99)
            spare = np.minimum.accumulate(
                np.where(dls > g, rcum[np.minimum(dls, n)] - rcum[g] - used - np.cumsum(due), np.inf))
            cands = []
            for key in keys:
                for it in streams[key][:8]:
                    if it.rel <= t and all(p.pos is not None and (p.pos + cfg['lat'] <= t or used >= r)
                                           for p in it.preds):
                        cands.append(it)
                        break
            if not cands:
                assert used < r
                used += r / 16
                continue
            ok = []
            for it in cands:
                j = int(np.searchsorted(dls, it.dl))
                if it.dl == cands[0].dl or j == 0 or spare[j - 1] >= it.cost.sum():
                    ok.append(it)
            it = min(ok, key=lambda it: np.max((cur + it.cost) / (cur + it.cost).sum()))
            if np.max(cur - hist + it.cost) > cfg['cap'] and spare[-1] >= r - used and used < r:
                break
            key = (it.dl,) + it.stage
            streams[key].remove(it)
            if not streams[key]:
                keys.remove(key)
            due[int(np.searchsorted(dls, it.dl))] -= it.cost.sum()
            it.pos = t
            used += it.cost.sum()
            cur = cur + it.cost
        debt = max(used - r, 0.0)
        hist = cur * cfg['decay']
    assert not keys


def schedule(L, cfg):
    morder = cfg['morder']
    off = -343 * L % 4
    ns = (343 * L + off) // 4
    slot = lambda G, k: (7 * G + k + off) // 4
    cost = lambda valu, ld, st: np.array([valu / 4, ld / 3, st * cfg['wst']])

    ca, cc = np.zeros((ns + 8, 3)), np.zeros((ns + 8, 3))
    for G in range(49 * L):
        i = morder[G % 7]
        lorder = cfg['lorder'][G % 4]
        T = len(AOP[i])
        seen = set()
        for j, k in enumerate(lorder):
            new = {g for _, g in AOP[k]} - seen
            seen |= new
            ca[slot(G, j)] += cost(4 + 8 * (len(AOP[k]) - 1) + 8 * (T - 1) * len(new), 8 + 8 * T * len(new), 0)
        nr = 0 if i in PRIMED else len(FIN[i][2]) + (2 if G // 7 % 7 == 2 else 0)
        for k, (_, _, rt) in FIN.items():
            arr = sorted(lorder.index(x) for x in [k] + [x for _, x in rt])
            for j in arr[1:]:
                cc[slot(G, j)] += cost(8, 0, 0)
            cc[slot(G, arr[-1])] += cost(8 * nr, 8 * nr, 8)
    lo = int(np.floor(cfg['shift']))
    fr = cfg['shift'] - lo
    fixed = cc[:ns] + (1 - fr) * ca[lo:lo + ns] + fr * ca[lo + 1:lo + ns + 1]

    done_at = {f: morder.index(i) for i, (f, _, _) in FIN.items()}
    items, reg = [], {}

    def build(kind, Q, l, rel0=None, dls=None):
        rel = [slot(49 * l + PH_DONE[Q] * 7 + done_at[f], 6) + 1 + cfg['w0'] for f in range(4)]
        use = slot(49 * l + PH_USE[Q] * 7, 0) - cfg['delay']
        x = 4 if Q == 2 else 0
        st = []
        if kind != 'init':
            nt = len(KT[Q][0])
            st.append(('K', [cost(4 * nt + 7, 4 * nt + 4, 4)] * 4))
        io = 4 if Q < 2 and l == 0 else 0
        st.append(('M', [{'init': cost(18, 4, 8) if Q >= 2 else cost(15, 4, 4),
                          'mix': cost(21 + x + 2 * io, 12 + x, 4 + io),
                          'final': cost(22 + x + (4 if Q >= 2 else 0), 12 + x, 4)}[kind]] * 4))
        if kind != 'final':
            v, ld, s = {0: (15, 8, 8), 1: (7, 4, 4), 2: (19, 12, 8), 3: (19, 12, 12)}[Q]
            st.append(('L', [cost(v + 7 * (s // 4 if f == 0 and Q != 1 else int(Q == 3)), ld, s) for f in range(4)]))
        for t in range(8 + len(st) - 1):
            for j in range(4):
                for si, (nm, c) in enumerate(st):
                    r = t - si
                    if not 0 <= r < 8:
                        continue
                    pre = [(kind, st[si - 1][0], Q, l, jj, r) for jj in range(4)] if si else []
                    if nm == 'M' and Q == 2:
                        pre += [(kind, 'K', 1, l, f, r) for f in range(4)]
                    if nm == 'L':
                        pre += [(kind, 'L', d, l, j, r) for d in {0: [1], 1: [], 3: [1, 0], 2: [1, 3]}[Q]]
                    rl = rel0[nm] if rel0 else (rel[j] if nm == 'K' else max(rel))
                    dl = min(dls[nm] if dls else use, ns - cfg['endm'])
                    if cfg['pace'] and Q == 3 and kind == 'init' and r < 4:
                        dl = dl * cfg['pace']
                    it = Item((kind, nm, Q, l), j, r, c[j], max(rl, 0), dl, [reg[k] for k in pre if k in reg])
                    reg[it.stage + (j, r)] = it
                    items.append(it)

    last = 49 * (L - 1)
    for Q in (3, 2):
        build('init', Q, -1, rel0=dict(M=0, L=0))
    for Q in (3, 2):
        build('final', Q, -1, dls=dict(K=slot(42, 0), M=slot(last, 0)))
    for l in range(L):
        for Q in (1, 0, 3, 2):
            if l < L - 1:
                build('mix', Q, l)
            elif Q < 2:
                build('final', Q, l, dls=dict(K=ns, M=ns))
    for Q in (1, 0):
        build('init', Q, L - 1, rel0=dict(M=slot(last, 0), L=slot(last + (14 if Q == 0 else 0), 0)), dls=dict(M=ns, L=ns))
    for it in items:
        kind, nm, Q, l = it.stage
        nxt, lead = {'K': ('M', cfg['leadk']), 'M': ('L', cfg['lead']), 'L': (None, 0)}[nm]
        k = (kind, nxt, Q, l, it.j, it.r - lead)
        if k in reg and reg[k].dl <= it.dl and reg[k].rel <= it.rel:
            it.preds.append(reg[k])
    place(items, fixed, cfg)
    stages = {}
    for it in items:
        stages.setdefault(it.stage, []).append(it)
    order = sorted(stages, key=lambda s: (max(it.pos for it in stages[s]), 'KML'.index(s[1])))
    anchor = lambda it: (max(min(4 * int(it.pos) + cfg['ak'] - off, 343 * L - 1), 0), min(int(it.pos % 1 * 8), 7))
    return [(s, {(it.j, it.r): anchor(it) for it in stages[s]}) for s in order]


def _kernel(x_hbm, ws_hbm, bs_hbm, o_hbm, z_ref, buf_ref, t_ref, bt_ref, bp_ref, w_ref, xf_ref, xb_ref, xin_ref,
            ost_ref, bs_ref, sem, *, cfg):
    L = bs_ref.shape[0]
    B, D = x_hbm.shape
    NC = D // 128
    nt = B // TM
    A4, ROWS = pl.ds(0, 4), pl.ds(0, RL)
    env = {}

    def enter(i):
        z = z_ref[0]
        env.update(z=z, buf=buf_ref.at[z], xc=xin_ref.at[i & 3], xp=xin_ref.at[(i + 3) & 3], o=ost_ref.at[i & 1],
                   true={}, ver=None, first={})

    def anchored(v, tok):
        if tok is None:
            return v
        if tok.shape not in env['true']:
            env['true'][tok.shape] = jnp.full(tok.shape, env['z'], jnp.int32) == 0
        return lax.select(env['true'][tok.shape], v if hasattr(v, 'shape') else jnp.full(tok.shape, v, F32), tok)

    def ld(it, f, g, ver):
        if env['ver'] is not None:
            for key in [(it, ff) for ff in (range(4) if f is A4 else [f])]:
                if key not in env['ver']:
                    env['ver'][key] = env['first'][key] = ver
                assert env['ver'][key] == ver, (key, ver)
        return env['buf'][it, f, g, ROWS]

    def st(it, f, g, ver, val):
        if env['ver'] is not None:
            env['ver'].update({(it, ff): ver for ff in (range(4) if f is A4 else [f])})
        env['buf'][it, f, g, ROWS] = val

    def io_idx(Q, q, p):
        r, c = bits(Q, q, p)
        return pl.ds((r ^ 4) * RL, RL), pl.ds(c * 128, 128)

    def scaled(v, Q, q, sign):
        lam = [(LAM[Q] * LAM[q] * LAM[p]) ** sign for p in range(len(v))]
        return [x if x is None or abs(s - 1) < 1e-9 else x * s for x, s in zip(v, lam)]

    def pass_k(Q, l, tok):
        terms, dst = KT[Q]
        e = [lin([(c, ld(it[l % 2], A4, g, l)) for c, it in terms]) for g in range(4)]
        c = c_tr(*e, anchored(0.5, tok))
        if l != 0:
            c = [c[p] + ld(dst[(l - 1) % 2], A4, p, l - 1) for p in range(4)]
        for p in range(4):
            st(dst[2 if l % L == L - 1 else l % 2], A4, p, l, c[p])

    def new_x(Q, l, tok, ps=A4):
        par = 2 if l % L == L - 1 else l % 2
        e = [ld(KT[Q][1][par], f, ps, l) for f in range(4)]
        if Q == 2:
            e = [e[f] + ld(DD[par], f, ps, l) for f in range(4)]
        c = c_tr(*e, anchored(0.5, tok))
        res = []
        for q in range(4):
            if l == (0 if Q < 2 else -1):
                x0 = stack([env['xp'][io_idx(Q, q, p)].astype(F32) for p in range(ps.start, ps.start + ps.size)])
                if Q < 2:
                    x0 = anchored(x0, tok)
                    st(X0[Q], q, A4, 0, x0)
            else:
                x0 = ld(X0[Q], q, ps, 0)
            b = jnp.concatenate([bt_ref[l % L, Q, q, ps]] * (RL // 8), axis=1)
            res.append((c[q] + b) * x0)
        return res

    def put_y(Q, l, x):
        for f, y in enumerate(a_tr(*x)):
            st(YY[Q], f, A4, l, y)

    def pass_init(Q, l, tok):
        x = []
        for q in range(4):
            v = [env['xc'][io_idx(Q, q, p)].astype(F32) for p in range(4)]
            if tok is not None and (Q >= 2 or q == 0):
                v = [anchored(v[p], tok[p]) for p in range(4)]
            if Q >= 2:
                st(X0[Q], q, A4, 0, stack(v))
            x.append(stack(scaled(v, Q, q, 1)))
        put_y(Q, l, x)

    def pass_final(Q, l, tok, ps=A4):
        for q, x in enumerate(new_x(Q, l, tok, ps)):
            x = [None] * ps.start + [x[k] for k in range(ps.size)]
            for p, v in enumerate(scaled(x, Q, q, -1)):
                if v is not None:
                    env['o'][io_idx(Q, q, p)] = v.astype(BF16)

    def pass_l(Q, l, tok):
        y = [ld(YY[Q], A4, p, l) for p in range(4)]
        v = a_tr(anchored(y[0], tok), *y[1:])
        get = lambda it: [ld(it, A4, g, l) for g in range(4)]
        add = lambda a, b: [p + q for p, q in zip(a, b)]
        sub = lambda a, b: [p - q for p, q in zip(a, b)]
        ss = SS[(l + 1) % 2]
        if Q == 1:
            out = {ss: v}
        elif Q == 0:
            s = get(ss)
            out = {NN: sub(v, s), PP: add(v, s)}
        elif Q == 3:
            s = get(ss)
            up = add(v, s)
            out = {TR: add(up, get(NN)), UP: up, UM: sub(v, s)}
        else:
            w, tr = add(v, get(ss)), get(TR)
            out = {GP: add(tr, w), GM: sub(tr, w)}
        for it, x in out.items():
            if Q != 1:
                h = x if it == TR else [u[:1] for u in x]
                r = h[0].astype(BF16).astype(F32)
                e2 = (r - h[0]) * 0.5
                h = [r] + [u + e2 for u in h[1:]]
                x = h if it == TR else [jnp.concatenate([a, u[1:]], axis=0) for a, u in zip(h, x)]
            for g in range(4):
                st(it, A4, g, l, x[g])

    def run_stage(stage, tok):
        kind, nm, Q, l = stage
        if nm == 'K':
            pass_k(Q, l, tok)
        elif nm == 'L':
            pass_l(Q, l, tok)
        elif kind == 'init':
            pass_init(Q, l, tok)
        elif kind == 'final':
            pass_final(Q, l, tok)
        else:
            put_y(Q, l, new_x(Q, l, tok))

    def group(G):
        l, ph, i, lorder = G // 49, G // 7 % 7, cfg['morder'][G % 7], cfg['lorder'][G % 4]
        I, src, dst = [(M3, NN, R3), (M5, PP, R5), (M1, TR, HH), (M4, UP, R4), (M7, UM, R7), (M2, GP, R2),
                       (M6, GM, R6)][ph]
        tmp, tver = TMP[(l * 7 + ph) % 2], l + ph / 8
        fs = [lin([(c, ld(src, f, g, l - 1)) for c, f in AOP[i]]) for g in range(4)]
        w = pltpu.bitcast(t_ref.bitcast(U32)[l, I * 7 + i], BF16)
        n = {}
        for k in lorder:
            op = lin([(c, fs[g]) for c, g in AOP[k]]).astype(BF16)
            n[k] = jnp.dot(op, w[k * 128:(k + 1) * 128], preferred_element_type=F32)
        e = [None] * 4
        for k, (f, sg, rt) in FIN.items():
            terms = dict([(k, sg)] + [(x, c) for c, x in rt])
            e[f] = lin([(terms[j], n[j]) for j in lorder if j in terms])
        e = stack(e)
        if i in PRIMED:
            st(tmp, PRIMED.index(i), A4, tver, e)
        else:
            f, sg, rt = FIN[i]
            so = -1 if I == M1 else 1
            terms = [(so * sg, e)] + [(so * c, ld(tmp, PRIMED.index(k), A4, tver)) for c, k in rt]
            if I == M1:
                terms += [(1, ld(it[l % 2], f, A4, l)) for it in (R3, R5)]
            st(dst[l % 2], f, A4, l, lin(terms))
        return [n[k] for k in lorder]

    def rows(r, n):
        return pl.ds(pl.multiple_of(r, HALF), n)

    def top_copy(i):
        return pltpu.make_async_copy(ost_ref.at[jnp.where(i == 1, 2, (i + 1) & 1), pl.ds(HALF, HALF)],
                                     o_hbm.at[rows(jnp.where(i == 1, B - HALF, (i - 2) * TM + HALF), HALF)], sem.at[4])

    def main_body(i, carry):
        enter(i)
        env['ver'] = {}
        copies = [
            pltpu.make_async_copy(x_hbm.at[rows(jnp.minimum(i + 1, nt - 1) * TM, TM)], xin_ref.at[(i + 1) & 3], sem.at[2]),
            top_copy(i),
            pltpu.make_async_copy(ost_ref.at[jnp.where(i == 1, 2, i & 1), pl.ds(0, HALF)],
                                  o_hbm.at[rows((i - 1) * TM, HALF)], sem.at[3])]
        copies[0].start()
        copies[1].start()
        todo = schedule(L, cfg)
        toks = []
        for G in range(49 * L):
            if G == 49 * (L - 1) + 3:
                assert all(stage[3] >= 0 for stage, _ in todo)
                copies[2].start()
            toks += group(G)
            while todo and max(p for p, _ in todo[0][1].values()) < len(toks):
                stage, anchors = todo.pop(0)
                tok = [toks[p][8 * r:8 * r + 8] for _, (p, r) in sorted(anchors.items())]
                run_stage(stage, jnp.concatenate(tok, axis=0).reshape(4, RL, 128))
        assert not todo and all(env['ver'][k] == v + L for k, v in env['first'].items())
        for c in copies:
            c.wait()
        return carry

    def w_start(l, slot):
        for c in range(NC):
            pltpu.make_async_copy(ws_hbm.at[l, :, pl.ds(c * 128, 128)], w_ref.at[slot, c], sem.at[slot]).start()

    def w_wait(slot):
        pltpu.make_async_copy(w_ref.at[slot], w_ref.at[slot], sem.at[slot]).wait()

    def second_block():
        return pltpu.make_async_copy(x_hbm.at[pl.ds(TM, TM)], xin_ref.at[1], sem.at[2])

    def pro_layer(l, carry):
        enter(0)
        slot = l & 1
        wu = w_ref.bitcast(U32).at[slot]
        xb, xu = xb_ref.at[env['z']], xb_ref.bitcast(U32).at[env['z']]
        toks = []
        for m in range(TM // RL):
            rs = pl.ds(m * RL, RL)
            xb[:, rs] = xf_ref[:, rs].astype(BF16)
            for n in range(NC):
                cols = pl.ds(n * 128, 128)
                lhs = pltpu.bitcast(xu[:, pl.ds(m * RL // 2, RL // 2)].reshape(NC * RL // 2, 128), BF16)
                lhs = [jnp.concatenate([lhs[c * RL:(c + 1) * RL] for c in range(h, h + NC // 2)], axis=1)
                       for h in (0, NC // 2)]
                w = pltpu.bitcast(wu[n], BF16)
                y1 = jnp.dot(lhs[0], w[:D // 2], preferred_element_type=F32)
                y2 = y1 + jnp.dot(lhs[1], w[D // 2:], preferred_element_type=F32)
                toks += [y1, y2]
                xf_ref[n, rs] = env['xp'][rs, cols].astype(F32) * (y2 + bp_ref[l, pl.ds(0, 1), cols]) + xf_ref[n, rs]

        buf = env['buf']
        blk = lambda it, f, g: (pl.ds(2 * it, 2), f, g, ROWS)
        dev = lambda k: blk(10, k // 4, k % 4)

        def rnd(x):
            x4 = x.reshape(8, 2, 8, 128)
            r = jnp.concatenate([x4[:, 0], x4[:, 1]], axis=2).astype(BF16).astype(F32)
            return jnp.stack([r[:, :, :128], r[:, :, 128:]], axis=1).reshape(x.shape)

        def w1(q, p, tok):
            v = []
            for Q in range(4):
                r, c = bits(Q, q, p)
                sc = -0.5 * LAM[Q] * LAM[q] * LAM[p]
                wb = pltpu.bitcast(wu[c, pl.ds(r * 64, 64)], BF16).astype(F32).reshape(2, RL, 128)
                v.append(wb * (anchored(sc, tok) if Q == 0 else sc))
            b11, s, t, b22 = v
            tr = b11 + b22
            for F, x in enumerate([tr, b11 - s, b11 + s, tr + (s + t), tr + tr]):
                buf[blk(F, q, p)] = x

        def w2(F, p, tok):
            y = [buf[blk(F, q, p)] for q in range(4)]
            for f, x in enumerate(a_tr(anchored(y[0], tok), *y[1:])):
                buf[blk(5 + F, f, p)] = x

        def w3(I, i, tok):
            b11, s, t, b22 = [lin([(c * C, buf[blk(5 + F, f, p)]) for C, F in BOP_OUT[I] for c, f in BOP[i]])
                              for p in range(4)]
            half = anchored(0.5, tok)
            tr = b11 + b22
            child = I == M1 and i != M1
            if child:
                tr, b11 = tr + buf[dev(0)], b11 + buf[dev(7)]
            r = rnd(tr)
            e2 = (r - tr) * half
            b11 = b11 + e2
            g = (r + (s + t)) * half
            o2, o6 = b11 - s, b11 + s
            out = [tr, o2, r - o6, r - g, r - o2, o6, g]
            if child:
                out = out[:1] + [out[k] + buf[dev(k)] for k in range(1, 7)]
            if I == M1 and i == M1:
                buf[dev(0)], buf[dev(7)] = e2, e2 * 0.5
                for k in range(1, 7):
                    buf[dev(k)] = (rnd(out[k]) - out[k]) * 0.5
            t_ref[l, I * 7 + i] = jnp.concatenate(out, axis=0).reshape(7 * 128, 128).astype(BF16)

        cost = lambda valu, ld_, st_: valu / 4 + ld_ / 3 + st_
        groups = sorted([(j / 42, 1 + j // 7, j % 7) for j in range(42)]
                        + [(0.2 + 0.8 * (j + .5) / 6, M1, j + 1) for j in range(6)] + [(-1, M1, M1)])
        passes = [[(cost(30, 8, 10), w1, q, p) for q in range(4) for p in range(4)],
                  [(cost(14, 8, 8), w2, F, p) for F in range(5) for p in range(4)], []]
        for _, I, i in groups:
            T = len(BOP_OUT[I]) * len(BOP[i])
            x = (0, 0, 0) if I != M1 else ((38, 0, 16) if i == M1 else (16, 16, 0))
            passes[2].append((cost(8 * (T - 1) + 33 + x[0], 8 * T + x[1], 7 + x[2]), w3, I, i))
        seq = sorted((rp + si + j / len(ps), si, j, rp) for si, ps in enumerate(passes) for j in range(len(ps))
                     for rp in range(8))
        fixed = np.zeros(len(toks))
        fixed[1::2] += cost(40, 24, 8)
        for o in range(2):
            fixed[(cfg['po'] + o) % 16::16] += cost(16, 32, 16)
        cum = np.concatenate([[0], np.cumsum(np.maximum(water(fixed, 8 * sum(e[0] for ps in passes for e in ps)) - fixed, 0))])
        where, acc = {}, 0.0
        for _, si, j, rp in seq:
            k = min(int(np.searchsorted(cum, acc, side='right')) - 1, len(toks) - 1)
            where[si, j, rp] = (k, min(int((acc - cum[k]) / (cum[k + 1] - cum[k]) * 8), 7))
            acc += passes[si][j][0]
        for si, ps in enumerate(passes):
            for j, (_, fn, a, b) in enumerate(ps):
                tok = [toks[k][8 * r:8 * r + 8] for k, r in (where[si, j, rp] for rp in range(8))]
                fn(a, b, jnp.concatenate([t for t in tok for _ in range(2)], axis=0).reshape(2, RL, 128))

        pl.when(l + 2 < L)(lambda: w_start(l + 2, slot))
        pl.when(l + 2 == L)(lambda: second_block().start())
        pl.when(l + 1 < L)(lambda: w_wait(1 - slot))
        return carry

    def prologue():
        z_ref[0] = 0
        first = [pltpu.make_async_copy(bs_hbm, bs_ref, sem.at[1]),
                 pltpu.make_async_copy(x_hbm.at[pl.ds(0, HALF)], xin_ref.at[3, pl.ds(0, HALF)], sem.at[2]),
                 pltpu.make_async_copy(x_hbm.at[pl.ds(B - HALF, HALF)], xin_ref.at[3, pl.ds(HALF, HALF)], sem.at[3]),
                 pltpu.make_async_copy(x_hbm.at[pl.ds(HALF, HALF)], xin_ref.at[0, pl.ds(HALF, HALF)], sem.at[4])]
        for c in first:
            c.start()
        w_start(0, 0)
        first[0].wait()
        beta = [jnp.ones((8, D), F32)]
        for l in range(L):
            bp_ref[l] = jnp.broadcast_to(bs_ref[l:l + 1, :].astype(F32), (8, D))
            beta.append(beta[-1] + bp_ref[l])
        beta = stack(beta[1:])
        for Q in range(4):
            for q in range(4):
                cols = [bits(Q, q, p)[1] * 128 for p in range(4)]
                for p, v in enumerate(scaled([beta[:, :, c:c + 128] for c in cols], Q, q, 1)):
                    bt_ref[:, Q, q, p] = v
        for c in first[1:]:
            c.wait()
        enter(0)
        x0 = env['xp'][...].astype(F32)
        for c in range(NC):
            xf_ref[c, pl.ds(0, TM)] = x0[:, c * 128:(c + 1) * 128]
        for Q in (1, 0):
            pass_init(Q, -1, None)
            pass_l(Q, -1, None)
        w_wait(0)
        w_start(1, 1)
        lax.fori_loop(0, L, pro_layer, 0)
        ost_ref[2] = jnp.concatenate([xf_ref[c, pl.ds(0, TM)] for c in range(NC)], axis=1).astype(BF16)
        second_block().wait()

    def drain():
        enter(nt)
        copies = [top_copy(jnp.int32(nt))]
        copies[0].start()
        for Q in (3, 2):
            pass_k(Q, -1, None)
        for h in range(2):
            for Q in (3, 2):
                pass_final(Q, -1, None, pl.ds(2 * h, 2))
            for j in range(2):
                r = (2 * j + h) * RL
                copies.append(pltpu.make_async_copy(ost_ref.at[nt % 2, pl.ds(r, RL)], o_hbm.at[pl.ds(B - TM + r, RL)],
                                                    sem.at[2 * h + j]))
                copies[-1].start()
        for c in copies:
            c.wait()

    prologue()
    lax.fori_loop(1, nt, main_body, 0)
    drain()


@jax.jit
def pallas_standalone__dcn_v2_cross__recsys_kernel(x0, ws, bs):
    B, D = x0.shape
    L = ws.shape[0]
    assert D == 1024 and L % 2 == 0 and B % TM == 0 and B >= 2 * TM
    cfg = dict(CFG)
    cfg.update(morder=[int(c) - 1 for c in str(cfg['mo'])], lorder=[[int(c) - 1 for c in o] for o in (str(cfg['lo']).split('x') * 4)[:4]])
    any_spec = pl.BlockSpec(memory_space=pl.ANY)
    return pl.pallas_call(
        functools.partial(_kernel, cfg=cfg),
        in_specs=[any_spec] * 3,
        out_specs=any_spec,
        out_shape=jax.ShapeDtypeStruct((B, D), x0.dtype),
        scratch_shapes=[
            pltpu.SMEM((1,), jnp.int32),
            pltpu.VMEM((1, NI, 5, 5, RL + 8, 128), F32),
            pltpu.VMEM((L, 49, 7 * 128, 128), BF16),
            pltpu.VMEM((L, 4, 4, 4, 8, 128), F32),
            pltpu.VMEM((L, 8, D), F32),
            pltpu.VMEM((2, D // 128, D, 128), BF16),
            pltpu.VMEM((D // 128, TM + 8, 128), F32),
            pltpu.VMEM((1, D // 128, TM, 128), BF16),
            pltpu.VMEM((4, TM, D), BF16),
            pltpu.VMEM((3, TM, D), BF16),
            pltpu.VMEM((L, D), BF16),
            pltpu.SemaphoreType.DMA((5,)),
        ],
        compiler_params=pltpu.CompilerParams(vmem_limit_bytes=127 * 1024 * 1024, disable_bounds_checks=True),
    )(x0, ws, bs)
```

```python
import functools

import numpy as np
import jax
import jax.numpy as jnp
from jax import lax
import jax.experimental.pallas as pl
import jax.experimental.pallas.tpu as pltpu

F32 = jnp.float32
BF16 = jnp.bfloat16
U32 = jnp.uint32

M1, M2, M3, M4, M5, M6, M7 = range(7)
SQ3 = float(np.sqrt(3.0))
LAM = (1.0, 1 / SQ3, SQ3, 1.0)
RL = 64
HALF = 4 * RL
TM = 2 * HALF
AOP = {M1: [(1, 0)], M3: [(1, 1)], M4: [(1, 0), (-1, 1)], M5: [(1, 2)], M7: [(1, 0), (-1, 2)],
       M2: [(1, 3)], M6: [(1, 0), (-1, 3)]}
BOP = {M1: [(1, 0)], M2: [(1, 1)], M5: [(1, 0), (-1, 1)], M6: [(1, 2)], M3: [(1, 0), (-1, 2)],
       M7: [(1, 3)], M4: [(1, 0), (-1, 3)]}
BOP_OUT = {**BOP, M1: [(1, 4)], M4: [(1, 4), (-1, 3)]}
PRIMED = [M5, M2, M6]
FIN = {M1: (0, -1, [(1, M5), (1, M2), (1, M6)]), M4: (1, 1, [(-1, M2)]), M7: (2, 1, [(-1, M6)]),
       M3: (3, 1, [(-1, M5)])}

GP, GM, TR, UP, UM = range(5)
TMP = [5, 6]
X0 = [7, 8, 9, 10]
R3, R5 = [11, 11], [12, 12]
HH, R4, R7, R2, R6 = [13, 14], [15, 16], [17, 18], [19, 20], [21, 22]
DD, C22, ZZ, C11 = [23, 24, 25], [26, 27, 28], [29, 30, 31], [32, 33, 33]
YY = [34, 35, 36, 37]
SS = [38, 39]
NN, PP = 40, 41
NI = 44
KT = {1: ([(1, R3), (-1, R5)], DD), 0: ([(1, HH), (1, R4), (1, R7)], C11),
      3: ([(1, HH), (1, R2), (1, R6)], C22), 2: ([(1, R4), (-1, R7), (-1, R2), (1, R6)], ZZ)}
PH_DONE = {1: 1, 0: 4, 3: 6, 2: 6}
PH_USE = {1: 7, 0: 7, 3: 9, 2: 12}

CFG = dict(mo=6254371, lo='2675341x2675431x5762431x1267543', delay=2.0, w0=0.5, shift=2.25, lat=0.15, slack=1.01,
           endm=0, wst=1.2, cap=56, decay=0, lead=2, leadk=3, pace=0.5, seg=8,
           jit='57557b25555555355515538545555555559a800555b1151555555055a55554155',
           po=14, l1=1.33, s1=0.75, l2=1.0, s2=1.0, pa=1.2, pb=0.75)


def lin(terms):
    k = next(i for i, t in enumerate(terms) if t[0] > 0)
    acc = terms[k][1]
    for i, (c, v) in enumerate(terms):
        if i != k:
            acc = acc + v if c > 0 else acc - v
    return acc


def a_tr(a11, s, t, a22):
    tr = a11 + a22
    return [tr, a11 - s, a11 + s, (tr + (s + t)) * 0.5]


def c_tr(e0, e1, e2, e3, half):
    h = e3 * half
    c22 = e0 + h
    return [(c22 + e1) + e2, h, (h + e1) - e2, c22]


def bits(Q, q, p):
    return (Q // 2) * 4 + (q // 2) * 2 + p // 2, (Q % 2) * 4 + (q % 2) * 2 + p % 2


def stack(xs):
    return jnp.concatenate(xs, axis=0).reshape((len(xs),) + xs[0].shape)


class Item:
    def __init__(self, stage, j, r, cost, rel, dl, preds):
        self.stage, self.j, self.r, self.cost, self.rel, self.dl, self.preds = stage, j, r, cost, rel, dl, preds
        self.pos = None


def water(fixed, work):
    f = np.sort(fixed)
    if len(f) == 0:
        return np.inf
    lv = (work + np.cumsum(f)) / np.arange(1, len(f) + 1)
    return lv[np.nonzero(lv >= f)[0][-1]]


def place(items, fixedv, cfg):
    fixed = fixedv.sum(1)
    n = len(fixed)
    jobs = {}
    for it in items:
        it.dl = int(np.floor(it.dl))
        k = (int(np.ceil(it.rel)), it.dl)
        jobs[k] = jobs.get(k, 0.0) + it.cost.sum()
    free = np.ones(n, bool)
    room = np.zeros(n)
    while jobs:
        best = None
        for a in sorted({k[0] for k in jobs}):
            for b in sorted({k[1] for k in jobs}):
                w = sum(v for k, v in jobs.items() if k[0] >= a and k[1] <= b)
                if b > a and w > 0:
                    lv = water(fixed[a:b][free[a:b]], w)
                    if best is None or lv > best[0]:
                        best = (lv, a, b)
        lv, a, b = best
        idx = np.arange(a, b)[free[a:b]]
        room[idx] = np.maximum(lv - fixed[idx], 0)
        free[a:b] = False
        jobs = {k: v for k, v in jobs.items() if not (k[0] >= a and k[1] <= b)}
    room = room * cfg['slack']
    rcum = np.concatenate([[0], np.cumsum(room)])
    dls = np.array(sorted({it.dl for it in items}))
    due = np.array([sum(it.cost.sum() for it in items if it.dl == d) for d in dls])
    streams = {}
    for it in items:
        streams.setdefault((it.dl,) + it.stage, []).append(it)
    keys = sorted(streams)
    debt = 0.0
    hist = np.zeros(3)
    for g in range(n):
        used = debt
        r = room[g]
        cur = fixedv[g] + hist
        while keys and (used < r or keys[0][0] <= g + 1):
            t = g + min(used / max(r, 1e-9), 0.99)
            spare = np.minimum.accumulate(
                np.where(dls > g, rcum[np.minimum(dls, n)] - rcum[g] - used - np.cumsum(due), np.inf))
            cands = []
            for key in keys:
                for it in streams[key][:8]:
                    if it.rel <= t and all(p.pos is not None and (p.pos + cfg['lat'] <= t or used >= r)
                                           for p in it.preds):
                        cands.append(it)
                        break
            if not cands:
                assert used < r
                used += r / 16
                continue
            ok = []
            for it in cands:
                j = int(np.searchsorted(dls, it.dl))
                if it.dl == cands[0].dl or j == 0 or spare[j - 1] >= it.cost.sum():
                    ok.append(it)
            it = min(ok, key=lambda it: np.max((cur + it.cost) / (cur + it.cost).sum()))
            if np.max(cur - hist + it.cost) > cfg['cap'] and spare[-1] >= r - used and used < r:
                break
            key = (it.dl,) + it.stage
            streams[key].remove(it)
            if not streams[key]:
                keys.remove(key)
            due[int(np.searchsorted(dls, it.dl))] -= it.cost.sum()
            it.pos = t
            used += it.cost.sum()
            cur = cur + it.cost
        debt = max(used - r, 0.0)
        hist = cur * cfg['decay']
    assert not keys


def schedule(L, cfg):
    morder = cfg['morder']
    off = -343 * L % 4
    ns = (343 * L + off) // 4
    slot = lambda G, k: (7 * G + k + off) // 4
    cost = lambda valu, ld, st: np.array([valu / 4, ld / 3, st * cfg['wst']])

    ca, cc = np.zeros((ns + 8, 3)), np.zeros((ns + 8, 3))
    for G in range(49 * L):
        i = morder[G % 7]
        lorder = cfg['lorder'][G % 4]
        T = len(AOP[i])
        seen = set()
        for j, k in enumerate(lorder):
            new = {g for _, g in AOP[k]} - seen
            seen |= new
            ca[slot(G, j)] += cost(4 + 8 * (len(AOP[k]) - 1) + 8 * (T - 1) * len(new), 8 + 8 * T * len(new), 0)
        nr = 0 if i in PRIMED else len(FIN[i][2]) + (2 if G // 7 % 7 == 2 else 0)
        for k, (_, _, rt) in FIN.items():
            arr = sorted(lorder.index(x) for x in [k] + [x for _, x in rt])
            for j in arr[1:]:
                cc[slot(G, j)] += cost(8, 0, 0)
            cc[slot(G, arr[-1])] += cost(8 * nr, 8 * nr, 8)
    lo = int(np.floor(cfg['shift']))
    fr = cfg['shift'] - lo
    fixed = cc[:ns] + (1 - fr) * ca[lo:lo + ns] + fr * ca[lo + 1:lo + ns + 1]

    done_at = {f: morder.index(i) for i, (f, _, _) in FIN.items()}
    items, reg = [], {}

    def build(kind, Q, l, rel0=None, dls=None):
        rel = [slot(49 * l + PH_DONE[Q] * 7 + done_at[f], 6) + 1 + cfg['w0'] for f in range(4)]
        use = slot(49 * l + PH_USE[Q] * 7, 0) - cfg['delay']
        x = 4 if Q == 2 else 0
        st = []
        if kind != 'init':
            nt = len(KT[Q][0])
            st.append(('K', [cost(4 * nt + 7, 4 * nt + 4, 4)] * 4))
        io = 4 if Q < 2 and l == 0 else 0
        st.append(('M', [{'init': cost(18, 4, 8) if Q >= 2 else cost(15, 4, 4),
                          'mix': cost(21 + x + 2 * io, 12 + x, 4 + io),
                          'final': cost(22 + x + (4 if Q >= 2 else 0), 12 + x, 4)}[kind]] * 4))
        if kind != 'final':
            v, ld, s = {0: (15, 8, 8), 1: (7, 4, 4), 2: (19, 12, 8), 3: (19, 12, 12)}[Q]
            st.append(('L', [cost(v + 7 * (s // 4 if f == 0 and Q != 1 else int(Q == 3)), ld, s) for f in range(4)]))
        for t in range(8 + len(st) - 1):
            for j in range(4):
                for si, (nm, c) in enumerate(st):
                    r = t - si
                    if not 0 <= r < 8:
                        continue
                    pre = [(kind, st[si - 1][0], Q, l, jj, r) for jj in range(4)] if si else []
                    if nm == 'M' and Q == 2:
                        pre += [(kind, 'K', 1, l, f, r) for f in range(4)]
                    if nm == 'L':
                        pre += [(kind, 'L', d, l, j, r) for d in {0: [1], 1: [], 3: [1, 0], 2: [1, 3]}[Q]]
                    rl = rel0[nm] if rel0 else (rel[j] if nm == 'K' else max(rel))
                    dl = min(dls[nm] if dls else use, ns - cfg['endm'])
                    if cfg['pace'] and Q == 3 and kind == 'init' and r < 4:
                        dl = dl * cfg['pace']
                    it = Item((kind, nm, Q, l), j, r, c[j], max(rl, 0), dl, [reg[k] for k in pre if k in reg])
                    reg[it.stage + (j, r)] = it
                    items.append(it)

    last = 49 * (L - 1)
    for Q in (3, 2):
        build('init', Q, -1, rel0=dict(M=0, L=0))
    for Q in (3, 2):
        build('final', Q, -1, dls=dict(K=slot(42, 0), M=slot(last, 0)))
    for l in range(L):
        for Q in (1, 0, 3, 2):
            if l < L - 1:
                build('mix', Q, l)
            elif Q < 2:
                build('final', Q, l, dls=dict(K=ns, M=ns))
    for Q in (1, 0):
        build('init', Q, L - 1, rel0=dict(M=slot(last, 0), L=slot(last + (14 if Q == 0 else 0), 0)), dls=dict(M=ns, L=ns))
    for it in items:
        kind, nm, Q, l = it.stage
        nxt, lead = {'K': ('M', cfg['leadk']), 'M': ('L', cfg['lead']), 'L': (None, 0)}[nm]
        k = (kind, nxt, Q, l, it.j, it.r - lead)
        if k in reg and reg[k].dl <= it.dl and reg[k].rel <= it.rel:
            it.preds.append(reg[k])
    place(items, fixed, cfg)
    stages = {}
    for it in items:
        stages.setdefault(it.stage, []).append(it)
    order = sorted(stages, key=lambda s: (max(it.pos for it in stages[s]), 'KML'.index(s[1])))

    def anchor(it):
        v = int(cfg['jit'][int(it.pos) // cfg['seg'] % len(cfg['jit'])], 16)
        t = min(max(int(it.pos * 8) + v // 4 - 1, 0), 8 * ns - 1)
        return max(min(4 * (t // 8) + v % 4 - off, 343 * L - 1), 0), t % 8
    return [(s, {(it.j, it.r): anchor(it) for it in stages[s]}) for s in order]


def _kernel(x_hbm, ws_hbm, bs_hbm, o_hbm, z_ref, buf_ref, t_ref, bt_ref, bp_ref, w_ref, xf_ref, xb_ref, xin_ref,
            ost_ref, bs_ref, sem, *, cfg):
    L = bs_ref.shape[0]
    B, D = x_hbm.shape
    NC = D // 128
    nt = B // TM
    A4, ROWS = pl.ds(0, 4), pl.ds(0, RL)
    env = {}

    def enter(i):
        z = z_ref[0]
        env.update(z=z, buf=buf_ref.at[z], xc=xin_ref.at[i & 3], xp=xin_ref.at[(i + 3) & 3], o=ost_ref.at[i & 1],
                   true={}, ver=None, first={})

    def anchored(v, tok):
        if tok is None:
            return v
        if tok.shape not in env['true']:
            env['true'][tok.shape] = jnp.full(tok.shape, env['z'], jnp.int32) == 0
        return lax.select(env['true'][tok.shape], v if hasattr(v, 'shape') else jnp.full(tok.shape, v, F32), tok)

    def ld(it, f, g, ver):
        if env['ver'] is not None:
            for key in [(it, ff) for ff in (range(4) if f is A4 else [f])]:
                if key not in env['ver']:
                    env['ver'][key] = env['first'][key] = ver
                assert env['ver'][key] == ver, (key, ver)
        return env['buf'][it, f, g, ROWS]

    def st(it, f, g, ver, val):
        if env['ver'] is not None:
            env['ver'].update({(it, ff): ver for ff in (range(4) if f is A4 else [f])})
        env['buf'][it, f, g, ROWS] = val

    def io_idx(Q, q, p):
        r, c = bits(Q, q, p)
        return pl.ds((r ^ 4) * RL, RL), pl.ds(c * 128, 128)

    def scaled(v, Q, q, sign):
        lam = [(LAM[Q] * LAM[q] * LAM[p]) ** sign for p in range(len(v))]
        return [x if x is None or abs(s - 1) < 1e-9 else x * s for x, s in zip(v, lam)]

    def pass_k(Q, l, tok):
        terms, dst = KT[Q]
        e = [lin([(c, ld(it[l % 2], A4, g, l)) for c, it in terms]) for g in range(4)]
        c = c_tr(*e, anchored(0.5, tok))
        if l != 0:
            c = [c[p] + ld(dst[(l - 1) % 2], A4, p, l - 1) for p in range(4)]
        for p in range(4):
            st(dst[2 if l % L == L - 1 else l % 2], A4, p, l, c[p])

    def new_x(Q, l, tok, ps=A4):
        par = 2 if l % L == L - 1 else l % 2
        e = [ld(KT[Q][1][par], f, ps, l) for f in range(4)]
        if Q == 2:
            e = [e[f] + ld(DD[par], f, ps, l) for f in range(4)]
        c = c_tr(*e, anchored(0.5, tok))
        res = []
        for q in range(4):
            if l == (0 if Q < 2 else -1):
                x0 = stack([env['xp'][io_idx(Q, q, p)].astype(F32) for p in range(ps.start, ps.start + ps.size)])
                if Q < 2:
                    x0 = anchored(x0, tok)
                    st(X0[Q], q, A4, 0, x0)
            else:
                x0 = ld(X0[Q], q, ps, 0)
            b = jnp.concatenate([bt_ref[l % L, Q, q, ps]] * (RL // 8), axis=1)
            res.append((c[q] + b) * x0)
        return res

    def put_y(Q, l, x):
        for f, y in enumerate(a_tr(*x)):
            st(YY[Q], f, A4, l, y)

    def pass_init(Q, l, tok):
        x = []
        for q in range(4):
            v = [env['xc'][io_idx(Q, q, p)].astype(F32) for p in range(4)]
            if tok is not None and (Q >= 2 or q == 0):
                v = [anchored(v[p], tok[p]) for p in range(4)]
            if Q >= 2:
                st(X0[Q], q, A4, 0, stack(v))
            x.append(stack(scaled(v, Q, q, 1)))
        put_y(Q, l, x)

    def pass_final(Q, l, tok, ps=A4):
        for q, x in enumerate(new_x(Q, l, tok, ps)):
            x = [None] * ps.start + [x[k] for k in range(ps.size)]
            for p, v in enumerate(scaled(x, Q, q, -1)):
                if v is not None:
                    env['o'][io_idx(Q, q, p)] = v.astype(BF16)

    def pass_l(Q, l, tok):
        y = [ld(YY[Q], A4, p, l) for p in range(4)]
        v = a_tr(anchored(y[0], tok), *y[1:])
        get = lambda it: [ld(it, A4, g, l) for g in range(4)]
        add = lambda a, b: [p + q for p, q in zip(a, b)]
        sub = lambda a, b: [p - q for p, q in zip(a, b)]
        ss = SS[(l + 1) % 2]
        if Q == 1:
            out = {ss: v}
        elif Q == 0:
            s = get(ss)
            out = {NN: sub(v, s), PP: add(v, s)}
        elif Q == 3:
            s = get(ss)
            up = add(v, s)
            out = {TR: add(up, get(NN)), UP: up, UM: sub(v, s)}
        else:
            w, tr = add(v, get(ss)), get(TR)
            out = {GP: add(tr, w), GM: sub(tr, w)}
        for it, x in out.items():
            if Q != 1:
                h = x if it == TR else [u[:1] for u in x]
                r = h[0].astype(BF16).astype(F32)
                e2 = (r - h[0]) * 0.5
                h = [r] + [u + e2 for u in h[1:]]
                x = h if it == TR else [jnp.concatenate([a, u[1:]], axis=0) for a, u in zip(h, x)]
            for g in range(4):
                st(it, A4, g, l, x[g])

    def run_stage(stage, tok):
        kind, nm, Q, l = stage
        if nm == 'K':
            pass_k(Q, l, tok)
        elif nm == 'L':
            pass_l(Q, l, tok)
        elif kind == 'init':
            pass_init(Q, l, tok)
        elif kind == 'final':
            pass_final(Q, l, tok)
        else:
            put_y(Q, l, new_x(Q, l, tok))

    def group(G):
        l, ph, i, lorder = G // 49, G // 7 % 7, cfg['morder'][G % 7], cfg['lorder'][G % 4]
        I, src, dst = [(M3, NN, R3), (M5, PP, R5), (M1, TR, HH), (M4, UP, R4), (M7, UM, R7), (M2, GP, R2),
                       (M6, GM, R6)][ph]
        tmp, tver = TMP[(l * 7 + ph) % 2], l + ph / 8
        fs = [lin([(c, ld(src, f, g, l - 1)) for c, f in AOP[i]]) for g in range(4)]
        w = pltpu.bitcast(t_ref.bitcast(U32)[l, I * 7 + i], BF16)
        n = {}
        for k in lorder:
            op = lin([(c, fs[g]) for c, g in AOP[k]]).astype(BF16)
            n[k] = jnp.dot(op, w[:, k * 16:(k + 1) * 16].reshape(128, 128), preferred_element_type=F32)
        e = [None] * 4
        for k, (f, sg, rt) in FIN.items():
            terms = dict([(k, sg)] + [(x, c) for c, x in rt])
            e[f] = lin([(terms[j], n[j]) for j in lorder if j in terms])
        e = stack(e)
        if i in PRIMED:
            st(tmp, PRIMED.index(i), A4, tver, e)
        else:
            f, sg, rt = FIN[i]
            so = -1 if I == M1 else 1
            terms = [(so * sg, e)] + [(so * c, ld(tmp, PRIMED.index(k), A4, tver)) for c, k in rt]
            if I == M1:
                terms += [(1, ld(it[l % 2], f, A4, l)) for it in (R3, R5)]
            st(dst[l % 2], f, A4, l, lin(terms))
        return [n[k] for k in lorder]

    def rows(r, n):
        return pl.ds(pl.multiple_of(r, HALF), n)

    def top_copy(i):
        return pltpu.make_async_copy(ost_ref.at[jnp.where(i == 1, 2, (i + 1) & 1), pl.ds(HALF, HALF)],
                                     o_hbm.at[rows(jnp.where(i == 1, B - HALF, (i - 2) * TM + HALF), HALF)], sem.at[4])

    def main_body(i, carry):
        enter(i)
        env['ver'] = {}
        copies = [
            pltpu.make_async_copy(x_hbm.at[rows(jnp.minimum(i + 1, nt - 1) * TM, TM)], xin_ref.at[(i + 1) & 3], sem.at[2]),
            top_copy(i),
            pltpu.make_async_copy(ost_ref.at[jnp.where(i == 1, 2, i & 1), pl.ds(0, HALF)],
                                  o_hbm.at[rows((i - 1) * TM, HALF)], sem.at[3])]
        copies[0].start()
        copies[1].start()
        todo = schedule(L, cfg)
        toks = []
        for G in range(49 * L):
            if G == 49 * (L - 1) + 3:
                assert all(stage[3] >= 0 for stage, _ in todo)
                copies[2].start()
            toks += group(G)
            while todo and max(p for p, _ in todo[0][1].values()) < len(toks):
                stage, anchors = todo.pop(0)
                tok = [toks[p][8 * r:8 * r + 8] for _, (p, r) in sorted(anchors.items())]
                run_stage(stage, jnp.concatenate(tok, axis=0).reshape(4, RL, 128))
        assert not todo and all(env['ver'][k] == v + L for k, v in env['first'].items())
        for c in copies:
            c.wait()
        return carry

    def w_start(l, slot):
        for c in range(NC):
            pltpu.make_async_copy(ws_hbm.at[l, :, pl.ds(c * 128, 128)], w_ref.at[slot, c], sem.at[slot]).start()

    def w_wait(slot):
        pltpu.make_async_copy(w_ref.at[slot], w_ref.at[slot], sem.at[slot]).wait()

    def second_block():
        return pltpu.make_async_copy(x_hbm.at[pl.ds(TM, TM)], xin_ref.at[1], sem.at[2])

    def pro_layer(l, carry):
        enter(0)
        slot = l & 1
        wu = w_ref.bitcast(U32).at[slot]
        xb, xu = xb_ref.at[env['z']], xb_ref.bitcast(U32).at[env['z']]
        toks = []
        for m in range(TM // RL):
            rs = pl.ds(m * RL, RL)
            xb[:, rs] = xf_ref[:, rs].astype(BF16)
            for n in range(NC):
                cols = pl.ds(n * 128, 128)
                lhs = pltpu.bitcast(xu[:, pl.ds(m * RL // 2, RL // 2)].reshape(NC * RL // 2, 128), BF16)
                lhs = [jnp.concatenate([lhs[c * RL:(c + 1) * RL] for c in range(h, h + NC // 2)], axis=1)
                       for h in (0, NC // 2)]
                w = pltpu.bitcast(wu[n], BF16)
                y1 = jnp.dot(lhs[0], w[:D // 2], preferred_element_type=F32)
                y2 = y1 + jnp.dot(lhs[1], w[D // 2:], preferred_element_type=F32)
                toks += [y1, y2]
                xf_ref[n, rs] = env['xp'][rs, cols].astype(F32) * (y2 + bp_ref[l, pl.ds(0, 1), cols]) + xf_ref[n, rs]

        buf = env['buf']
        blk = lambda it, f, g: (pl.ds(2 * it, 2), f, g, ROWS)
        dev = lambda k: blk(10, k // 4, k % 4)

        def rnd(x):
            x4 = x.reshape(8, 2, 8, 128)
            r = jnp.concatenate([x4[:, 0], x4[:, 1]], axis=2).astype(BF16).astype(F32)
            return jnp.stack([r[:, :, :128], r[:, :, 128:]], axis=1).reshape(x.shape)

        def w1(q, p, tok):
            v = []
            for Q in range(4):
                r, c = bits(Q, q, p)
                sc = -0.5 * LAM[Q] * LAM[q] * LAM[p]
                wb = pltpu.bitcast(wu[c, pl.ds(r * 64, 64)], BF16).astype(F32).reshape(2, RL, 128)
                v.append(wb * (anchored(sc, tok) if Q == 0 else sc))
            b11, s, t, b22 = v
            tr = b11 + b22
            for F, x in enumerate([tr, b11 - s, b11 + s, tr + (s + t), tr + tr]):
                buf[blk(F, q, p)] = x

        def w2(F, p, tok):
            y = [buf[blk(F, q, p)] for q in range(4)]
            for f, x in enumerate(a_tr(anchored(y[0], tok), *y[1:])):
                buf[blk(5 + F, f, p)] = x

        def w3(I, i, tok):
            b11, s, t, b22 = [lin([(c * C, buf[blk(5 + F, f, p)]) for C, F in BOP_OUT[I] for c, f in BOP[i]])
                              for p in range(4)]
            half = anchored(0.5, tok)
            tr = b11 + b22
            child = I == M1 and i != M1
            if child:
                tr, b11 = tr + buf[dev(0)], b11 + buf[dev(7)]
            r = rnd(tr)
            e2 = (r - tr) * half
            b11 = b11 + e2
            g = (r + (s + t)) * half
            o2, o6 = b11 - s, b11 + s
            out = [tr, o2, r - o6, r - g, r - o2, o6, g]
            if child:
                out = out[:1] + [out[k] + buf[dev(k)] for k in range(1, 7)]
            if I == M1 and i == M1:
                buf[dev(0)], buf[dev(7)] = e2, e2 * 0.5
                for k in range(1, 7):
                    buf[dev(k)] = (rnd(out[k]) - out[k]) * 0.5
            t_ref[l, I * 7 + i] = jnp.concatenate([x.reshape(8, 16, 128) for x in out], axis=1).astype(BF16)

        cost = lambda valu, ld_, st_: valu * cfg['pa'] / 4 + ld_ * cfg['pb'] / 3 + st_
        groups = sorted([(j / 42, 1 + j // 7, j % 7) for j in range(42)]
                        + [(0.2 + 0.8 * (j + .5) / 6, M1, j + 1) for j in range(6)] + [(-1, M1, M1)])
        passes = [[(cost(30, 4, 10), w1, q, p) for p in range(4) for q in range(4)],
                  [(cost(14, 8, 8), w2, F, p) for p in range(4) for F in range(5)], []]
        for _, I, i in groups:
            T = len(BOP_OUT[I]) * len(BOP[i])
            x = (0, 0, 0) if I != M1 else ((38, 0, 16) if i == M1 else (16, 16, 0))
            passes[2].append((cost(8 * (T - 1) + 33 + x[0], 8 * T + x[1], 7 + x[2]), w3, I, i))
        span = [(-cfg['l1'], cfg['s1']), (-cfg['l2'], cfg['s2']), (0, 1)]
        seq = sorted((rp + span[si][0] + span[si][1] * j / len(ps), si, j, rp) for si, ps in enumerate(passes)
                     for j in range(len(ps)) for rp in range(8))
        fixed = np.zeros(len(toks))
        fixed[1::2] += cost(40, 24, 8)
        for o in range(2):
            fixed[(cfg['po'] + o) % 16::16] += cost(16, 32, 16)
        cum = np.concatenate([[0], np.cumsum(np.maximum(water(fixed, 8 * sum(e[0] for ps in passes for e in ps)) - fixed, 0))])
        where, acc = {}, 0.0
        for _, si, j, rp in seq:
            k = min(int(np.searchsorted(cum, acc, side='right')) - 1, len(toks) - 1)
            where[si, j, rp] = (k, min(int((acc - cum[k]) / (cum[k + 1] - cum[k]) * 8), 7))
            acc += passes[si][j][0]
        for si, ps in enumerate(passes):
            for j, (_, fn, a, b) in enumerate(ps):
                tok = [toks[k][8 * r:8 * r + 8] for k, r in (where[si, j, rp] for rp in range(8))]
                fn(a, b, jnp.concatenate([t for t in tok for _ in range(2)], axis=0).reshape(2, RL, 128))

        pl.when(l + 2 < L)(lambda: w_start(l + 2, slot))
        pl.when(l + 2 == L)(lambda: second_block().start())
        pl.when(l + 1 < L)(lambda: w_wait(1 - slot))
        return carry

    def prologue():
        z_ref[0] = 0
        first = [pltpu.make_async_copy(bs_hbm, bs_ref, sem.at[1]),
                 pltpu.make_async_copy(x_hbm.at[pl.ds(0, HALF)], xin_ref.at[3, pl.ds(0, HALF)], sem.at[2]),
                 pltpu.make_async_copy(x_hbm.at[pl.ds(B - HALF, HALF)], xin_ref.at[3, pl.ds(HALF, HALF)], sem.at[3]),
                 pltpu.make_async_copy(x_hbm.at[pl.ds(HALF, HALF)], xin_ref.at[0, pl.ds(HALF, HALF)], sem.at[4])]
        for c in first:
            c.start()
        w_start(0, 0)
        first[0].wait()
        beta = [jnp.ones((8, D), F32)]
        for l in range(L):
            bp_ref[l] = jnp.broadcast_to(bs_ref[l:l + 1, :].astype(F32), (8, D))
            beta.append(beta[-1] + bp_ref[l])
        beta = stack(beta[1:])
        for Q in range(4):
            for q in range(4):
                cols = [bits(Q, q, p)[1] * 128 for p in range(4)]
                for p, v in enumerate(scaled([beta[:, :, c:c + 128] for c in cols], Q, q, 1)):
                    bt_ref[:, Q, q, p] = v
        for c in first[1:]:
            c.wait()
        enter(0)
        x0 = env['xp'][...].astype(F32)
        for c in range(NC):
            xf_ref[c, pl.ds(0, TM)] = x0[:, c * 128:(c + 1) * 128]
        for Q in (1, 0):
            pass_init(Q, -1, None)
            pass_l(Q, -1, None)
        w_wait(0)
        w_start(1, 1)
        lax.fori_loop(0, L, pro_layer, 0)
        ost_ref[2] = jnp.concatenate([xf_ref[c, pl.ds(0, TM)] for c in range(NC)], axis=1).astype(BF16)
        second_block().wait()

    def drain():
        enter(nt)
        copies = [top_copy(jnp.int32(nt))]
        copies[0].start()
        for Q in (3, 2):
            pass_k(Q, -1, None)
        for h in range(2):
            for Q in (3, 2):
                pass_final(Q, -1, None, pl.ds(2 * h, 2))
            for j in range(2):
                r = (2 * j + h) * RL
                copies.append(pltpu.make_async_copy(ost_ref.at[nt % 2, pl.ds(r, RL)], o_hbm.at[pl.ds(B - TM + r, RL)],
                                                    sem.at[2 * h + j]))
                copies[-1].start()
        for c in copies:
            c.wait()

    prologue()
    lax.fori_loop(1, nt, main_body, 0)
    drain()


@jax.jit
def pallas_standalone__dcn_v2_cross__recsys_kernel(x0, ws, bs):
    B, D = x0.shape
    L = ws.shape[0]
    assert D == 1024 and L % 2 == 0 and B % TM == 0 and B >= 2 * TM
    cfg = dict(CFG)
    cfg.update(morder=[int(c) - 1 for c in str(cfg['mo'])], lorder=[[int(c) - 1 for c in o] for o in (str(cfg['lo']).split('x') * 4)[:4]])
    any_spec = pl.BlockSpec(memory_space=pl.ANY)
    return pl.pallas_call(
        functools.partial(_kernel, cfg=cfg),
        in_specs=[any_spec] * 3,
        out_specs=any_spec,
        out_shape=jax.ShapeDtypeStruct((B, D), x0.dtype),
        scratch_shapes=[
            pltpu.SMEM((1,), jnp.int32),
            pltpu.VMEM((1, NI, 5, 5, RL + 8, 128), F32),
            pltpu.VMEM((L, 49, 8, 7 * 16, 128), BF16),
            pltpu.VMEM((L, 4, 4, 4, 8, 128), F32),
            pltpu.VMEM((L, 8, D), F32),
            pltpu.VMEM((2, D // 128, D, 128), BF16),
            pltpu.VMEM((D // 128, TM + 8, 128), F32),
            pltpu.VMEM((1, D // 128, TM, 128), BF16),
            pltpu.VMEM((4, TM, D), BF16),
            pltpu.VMEM((3, TM, D), BF16),
            pltpu.VMEM((L, D), BF16),
            pltpu.SemaphoreType.DMA((5,)),
        ],
        compiler_params=pltpu.CompilerParams(vmem_limit_bytes=127 * 1024 * 1024, disable_bounds_checks=True),
    )(x0, ws, bs)
```

```python
import functools

import numpy as np
import jax
import jax.numpy as jnp
from jax import lax
import jax.experimental.pallas as pl
import jax.experimental.pallas.tpu as pltpu

F32 = jnp.float32
BF16 = jnp.bfloat16
U32 = jnp.uint32

M1, M2, M3, M4, M5, M6, M7 = range(7)
SQ3 = float(np.sqrt(3.0))
LAM = (1.0, 1 / SQ3, SQ3, 1.0)
RL = 64
HALF = 4 * RL
TM = 2 * HALF
AOP = {M1: [(1, 0)], M3: [(1, 1)], M4: [(1, 0), (-1, 1)], M5: [(1, 2)], M7: [(1, 0), (-1, 2)],
       M2: [(1, 3)], M6: [(1, 0), (-1, 3)]}
BOP = {M1: [(1, 0)], M2: [(1, 1)], M5: [(1, 0), (-1, 1)], M6: [(1, 2)], M3: [(1, 0), (-1, 2)],
       M7: [(1, 3)], M4: [(1, 0), (-1, 3)]}
BOP_OUT = {**BOP, M1: [(1, 4)], M4: [(1, 4), (-1, 3)]}
PRIMED = [M5, M2, M6]
FIN = {M1: (0, -1, [(1, M5), (1, M2), (1, M6)]), M4: (1, 1, [(-1, M2)]), M7: (2, 1, [(-1, M6)]),
       M3: (3, 1, [(-1, M5)])}

GP, GM, TR, UP, UM = range(5)
TMP = [5, 6]
X0 = [7, 8, 9, 10]
R3, R5 = [11, 11], [12, 12]
HH, R4, R7, R2, R6 = [13, 14], [15, 16], [17, 18], [19, 20], [21, 22]
DD, C22, ZZ, C11 = [23, 24, 25], [26, 27, 28], [29, 30, 31], [32, 33, 33]
YY = [34, 35, 36, 37]
SS = [38, 39]
NN, PP = 40, 41
NI = 44
KT = {1: ([(1, R3), (-1, R5)], DD), 0: ([(1, HH), (1, R4), (1, R7)], C11),
      3: ([(1, HH), (1, R2), (1, R6)], C22), 2: ([(1, R4), (-1, R7), (-1, R2), (1, R6)], ZZ)}
PH_DONE = {1: 1, 0: 4, 3: 6, 2: 6}
PH_USE = {1: 7, 0: 7, 3: 9, 2: 12}

CFG = dict(mo=6254371, lo='2675341x2675431x5762431x1267543', delay=2.0, w0=0.5, shift=2.25, lat=0.15, slack=1.01,
           endm=0, wst=1.2, cap=56, decay=0, lead=2, leadk=3, pace=0.5, seg=8,
           jit='57557b25555555355512518545555855799a80015500151555555055a55554155',
           po=14, l1=1.17, s1=0.4, l2=1.05, s2=1.0, pa=0.92, pb=8, pe=-2)


def lin(terms):
    k = next(i for i, t in enumerate(terms) if t[0] > 0)
    acc = terms[k][1]
    for i, (c, v) in enumerate(terms):
        if i != k:
            acc = acc + v if c > 0 else acc - v
    return acc


def a_tr(a11, s, t, a22):
    tr = a11 + a22
    return [tr, a11 - s, a11 + s, (tr + (s + t)) * 0.5]


def c_tr(e0, e1, e2, e3, half):
    h = e3 * half
    c22 = e0 + h
    return [(c22 + e1) + e2, h, (h + e1) - e2, c22]


def bits(Q, q, p):
    return (Q // 2) * 4 + (q // 2) * 2 + p // 2, (Q % 2) * 4 + (q % 2) * 2 + p % 2


def stack(xs):
    return jnp.concatenate(xs, axis=0).reshape((len(xs),) + xs[0].shape)


class Item:
    def __init__(self, stage, j, r, cost, rel, dl, preds):
        self.stage, self.j, self.r, self.cost, self.rel, self.dl, self.preds = stage, j, r, cost, rel, dl, preds
        self.pos = None


def water(fixed, work):
    f = np.sort(fixed)
    if len(f) == 0:
        return np.inf
    lv = (work + np.cumsum(f)) / np.arange(1, len(f) + 1)
    return lv[np.nonzero(lv >= f)[0][-1]]


def place(items, fixedv, cfg):
    fixed = fixedv.sum(1)
    n = len(fixed)
    jobs = {}
    for it in items:
        it.dl = int(np.floor(it.dl))
        k = (int(np.ceil(it.rel)), it.dl)
        jobs[k] = jobs.get(k, 0.0) + it.cost.sum()
    free = np.ones(n, bool)
    room = np.zeros(n)
    while jobs:
        best = None
        for a in sorted({k[0] for k in jobs}):
            for b in sorted({k[1] for k in jobs}):
                w = sum(v for k, v in jobs.items() if k[0] >= a and k[1] <= b)
                if b > a and w > 0:
                    lv = water(fixed[a:b][free[a:b]], w)
                    if best is None or lv > best[0]:
                        best = (lv, a, b)
        lv, a, b = best
        idx = np.arange(a, b)[free[a:b]]
        room[idx] = np.maximum(lv - fixed[idx], 0)
        free[a:b] = False
        jobs = {k: v for k, v in jobs.items() if not (k[0] >= a and k[1] <= b)}
    room = room * cfg['slack']
    rcum = np.concatenate([[0], np.cumsum(room)])
    dls = np.array(sorted({it.dl for it in items}))
    due = np.array([sum(it.cost.sum() for it in items if it.dl == d) for d in dls])
    streams = {}
    for it in items:
        streams.setdefault((it.dl,) + it.stage, []).append(it)
    keys = sorted(streams)
    debt = 0.0
    hist = np.zeros(3)
    for g in range(n):
        used = debt
        r = room[g]
        cur = fixedv[g] + hist
        while keys and (used < r or keys[0][0] <= g + 1):
            t = g + min(used / max(r, 1e-9), 0.99)
            spare = np.minimum.accumulate(
                np.where(dls > g, rcum[np.minimum(dls, n)] - rcum[g] - used - np.cumsum(due), np.inf))
            cands = []
            for key in keys:
                for it in streams[key][:8]:
                    if it.rel <= t and all(p.pos is not None and (p.pos + cfg['lat'] <= t or used >= r)
                                           for p in it.preds):
                        cands.append(it)
                        break
            if not cands:
                assert used < r
                used += r / 16
                continue
            ok = []
            for it in cands:
                j = int(np.searchsorted(dls, it.dl))
                if it.dl == cands[0].dl or j == 0 or spare[j - 1] >= it.cost.sum():
                    ok.append(it)
            it = min(ok, key=lambda it: np.max((cur + it.cost) / (cur + it.cost).sum()))
            if np.max(cur - hist + it.cost) > cfg['cap'] and spare[-1] >= r - used and used < r:
                break
            key = (it.dl,) + it.stage
            streams[key].remove(it)
            if not streams[key]:
                keys.remove(key)
            due[int(np.searchsorted(dls, it.dl))] -= it.cost.sum()
            it.pos = t
            used += it.cost.sum()
            cur = cur + it.cost
        debt = max(used - r, 0.0)
        hist = cur * cfg['decay']
    assert not keys


def schedule(L, cfg):
    morder = cfg['morder']
    off = -343 * L % 4
    ns = (343 * L + off) // 4
    slot = lambda G, k: (7 * G + k + off) // 4
    cost = lambda valu, ld, st: np.array([valu / 4, ld / 3, st * cfg['wst']])

    ca, cc = np.zeros((ns + 8, 3)), np.zeros((ns + 8, 3))
    for G in range(49 * L):
        i = morder[G % 7]
        lorder = cfg['lorder'][G % 4]
        T = len(AOP[i])
        seen = set()
        for j, k in enumerate(lorder):
            new = {g for _, g in AOP[k]} - seen
            seen |= new
            ca[slot(G, j)] += cost(4 + 8 * (len(AOP[k]) - 1) + 8 * (T - 1) * len(new), 8 + 8 * T * len(new), 0)
        nr = 0 if i in PRIMED else len(FIN[i][2]) + (2 if G // 7 % 7 == 2 else 0)
        for k, (_, _, rt) in FIN.items():
            arr = sorted(lorder.index(x) for x in [k] + [x for _, x in rt])
            for j in arr[1:]:
                cc[slot(G, j)] += cost(8, 0, 0)
            cc[slot(G, arr[-1])] += cost(8 * nr, 8 * nr, 8)
    lo = int(np.floor(cfg['shift']))
    fr = cfg['shift'] - lo
    fixed = cc[:ns] + (1 - fr) * ca[lo:lo + ns] + fr * ca[lo + 1:lo + ns + 1]

    done_at = {f: morder.index(i) for i, (f, _, _) in FIN.items()}
    items, reg = [], {}

    def build(kind, Q, l, rel0=None, dls=None):
        rel = [slot(49 * l + PH_DONE[Q] * 7 + done_at[f], 6) + 1 + cfg['w0'] for f in range(4)]
        use = slot(49 * l + PH_USE[Q] * 7, 0) - cfg['delay']
        x = 4 if Q == 2 else 0
        st = []
        if kind != 'init':
            nt = len(KT[Q][0])
            st.append(('K', [cost(4 * nt + 7, 4 * nt + 4, 4)] * 4))
        io = 4 if Q < 2 and l == 0 else 0
        st.append(('M', [{'init': cost(18, 4, 8) if Q >= 2 else cost(15, 4, 4),
                          'mix': cost(21 + x + 2 * io, 12 + x, 4 + io),
                          'final': cost(22 + x + (4 if Q >= 2 else 0), 12 + x, 4)}[kind]] * 4))
        if kind != 'final':
            v, ld, s = {0: (15, 8, 8), 1: (7, 4, 4), 2: (19, 12, 8), 3: (19, 12, 12)}[Q]
            st.append(('L', [cost(v + 7 * (s // 4 if f == 0 and Q != 1 else int(Q == 3)), ld, s) for f in range(4)]))
        for t in range(8 + len(st) - 1):
            for j in range(4):
                for si, (nm, c) in enumerate(st):
                    r = t - si
                    if not 0 <= r < 8:
                        continue
                    pre = [(kind, st[si - 1][0], Q, l, jj, r) for jj in range(4)] if si else []
                    if nm == 'M' and Q == 2:
                        pre += [(kind, 'K', 1, l, f, r) for f in range(4)]
                    if nm == 'L':
                        pre += [(kind, 'L', d, l, j, r) for d in {0: [1], 1: [], 3: [1, 0], 2: [1, 3]}[Q]]
                    rl = rel0[nm] if rel0 else (rel[j] if nm == 'K' else max(rel))
                    dl = min(dls[nm] if dls else use, ns - cfg['endm'])
                    if cfg['pace'] and Q == 3 and kind == 'init' and r < 4:
                        dl = dl * cfg['pace']
                    it = Item((kind, nm, Q, l), j, r, c[j], max(rl, 0), dl, [reg[k] for k in pre if k in reg])
                    reg[it.stage + (j, r)] = it
                    items.append(it)

    last = 49 * (L - 1)
    for Q in (3, 2):
        build('init', Q, -1, rel0=dict(M=0, L=0))
    for Q in (3, 2):
        build('final', Q, -1, dls=dict(K=slot(42, 0), M=slot(last, 0)))
    for l in range(L):
        for Q in (1, 0, 3, 2):
            if l < L - 1:
                build('mix', Q, l)
            elif Q < 2:
                build('final', Q, l, dls=dict(K=ns, M=ns))
    for Q in (1, 0):
        build('init', Q, L - 1, rel0=dict(M=slot(last, 0), L=slot(last + (14 if Q == 0 else 0), 0)), dls=dict(M=ns, L=ns))
    for it in items:
        kind, nm, Q, l = it.stage
        nxt, lead = {'K': ('M', cfg['leadk']), 'M': ('L', cfg['lead']), 'L': (None, 0)}[nm]
        k = (kind, nxt, Q, l, it.j, it.r - lead)
        if k in reg and reg[k].dl <= it.dl and reg[k].rel <= it.rel:
            it.preds.append(reg[k])
    place(items, fixed, cfg)
    stages = {}
    for it in items:
        stages.setdefault(it.stage, []).append(it)
    order = sorted(stages, key=lambda s: (max(it.pos for it in stages[s]), 'KML'.index(s[1])))

    def anchor(it):
        v = int(cfg['jit'][int(it.pos) // cfg['seg'] % len(cfg['jit'])], 16)
        t = min(max(int(it.pos * 8) + v // 4 - 1, 0), 8 * ns - 1)
        return max(min(4 * (t // 8) + v % 4 - off, 343 * L - 1), 0), t % 8
    return [(s, {(it.j, it.r): anchor(it) for it in stages[s]}) for s in order]


def _kernel(x_hbm, ws_hbm, bs_hbm, o_hbm, z_ref, buf_ref, t_ref, bt_ref, bp_ref, w_ref, xf_ref, xb_ref, xin_ref,
            ost_ref, bs_ref, sem, *, cfg):
    L = bs_ref.shape[0]
    B, D = x_hbm.shape
    NC = D // 128
    nt = B // TM
    A4, ROWS = pl.ds(0, 4), pl.ds(0, RL)
    env = {}

    def enter(i):
        z = z_ref[0]
        env.update(z=z, buf=buf_ref.at[z], xc=xin_ref.at[i & 3], xp=xin_ref.at[(i + 3) & 3], o=ost_ref.at[i & 1],
                   true={}, ver=None, first={})

    def anchored(v, tok):
        if tok is None:
            return v
        if tok.shape not in env['true']:
            env['true'][tok.shape] = jnp.full(tok.shape, env['z'], jnp.int32) == 0
        return lax.select(env['true'][tok.shape], v if hasattr(v, 'shape') else jnp.full(tok.shape, v, F32), tok)

    def ld(it, f, g, ver):
        if env['ver'] is not None:
            for key in [(it, ff) for ff in (range(4) if f is A4 else [f])]:
                if key not in env['ver']:
                    env['ver'][key] = env['first'][key] = ver
                assert env['ver'][key] == ver, (key, ver)
        return env['buf'][it, f, g, ROWS]

    def st(it, f, g, ver, val):
        if env['ver'] is not None:
            env['ver'].update({(it, ff): ver for ff in (range(4) if f is A4 else [f])})
        env['buf'][it, f, g, ROWS] = val

    def io_idx(Q, q, p):
        r, c = bits(Q, q, p)
        return pl.ds((r ^ 4) * RL, RL), pl.ds(c * 128, 128)

    def scaled(v, Q, q, sign):
        lam = [(LAM[Q] * LAM[q] * LAM[p]) ** sign for p in range(len(v))]
        return [x if x is None or abs(s - 1) < 1e-9 else x * s for x, s in zip(v, lam)]

    def pass_k(Q, l, tok):
        terms, dst = KT[Q]
        e = [lin([(c, ld(it[l % 2], A4, g, l)) for c, it in terms]) for g in range(4)]
        c = c_tr(*e, anchored(0.5, tok))
        if l != 0:
            c = [c[p] + ld(dst[(l - 1) % 2], A4, p, l - 1) for p in range(4)]
        for p in range(4):
            st(dst[2 if l % L == L - 1 else l % 2], A4, p, l, c[p])

    def new_x(Q, l, tok, ps=A4):
        par = 2 if l % L == L - 1 else l % 2
        e = [ld(KT[Q][1][par], f, ps, l) for f in range(4)]
        if Q == 2:
            e = [e[f] + ld(DD[par], f, ps, l) for f in range(4)]
        c = c_tr(*e, anchored(0.5, tok))
        res = []
        for q in range(4):
            if l == (0 if Q < 2 else -1):
                x0 = stack([env['xp'][io_idx(Q, q, p)].astype(F32) for p in range(ps.start, ps.start + ps.size)])
                if Q < 2:
                    x0 = anchored(x0, tok)
                    st(X0[Q], q, A4, 0, x0)
            else:
                x0 = ld(X0[Q], q, ps, 0)
            b = jnp.concatenate([bt_ref[l % L, Q, q, ps]] * (RL // 8), axis=1)
            res.append((c[q] + b) * x0)
        return res

    def put_y(Q, l, x):
        for f, y in enumerate(a_tr(*x)):
            st(YY[Q], f, A4, l, y)

    def pass_init(Q, l, tok):
        x = []
        for q in range(4):
            v = [env['xc'][io_idx(Q, q, p)].astype(F32) for p in range(4)]
            if tok is not None and (Q >= 2 or q == 0):
                v = [anchored(v[p], tok[p]) for p in range(4)]
            if Q >= 2:
                st(X0[Q], q, A4, 0, stack(v))
            x.append(stack(scaled(v, Q, q, 1)))
        put_y(Q, l, x)

    def pass_final(Q, l, tok, ps=A4):
        for q, x in enumerate(new_x(Q, l, tok, ps)):
            x = [None] * ps.start + [x[k] for k in range(ps.size)]
            for p, v in enumerate(scaled(x, Q, q, -1)):
                if v is not None:
                    env['o'][io_idx(Q, q, p)] = v.astype(BF16)

    def pass_l(Q, l, tok):
        y = [ld(YY[Q], A4, p, l) for p in range(4)]
        v = a_tr(anchored(y[0], tok), *y[1:])
        get = lambda it: [ld(it, A4, g, l) for g in range(4)]
        add = lambda a, b: [p + q for p, q in zip(a, b)]
        sub = lambda a, b: [p - q for p, q in zip(a, b)]
        ss = SS[(l + 1) % 2]
        if Q == 1:
            out = {ss: v}
        elif Q == 0:
            s = get(ss)
            out = {NN: sub(v, s), PP: add(v, s)}
        elif Q == 3:
            s = get(ss)
            up = add(v, s)
            out = {TR: add(up, get(NN)), UP: up, UM: sub(v, s)}
        else:
            w, tr = add(v, get(ss)), get(TR)
            out = {GP: add(tr, w), GM: sub(tr, w)}
        for it, x in out.items():
            if Q != 1:
                h = x if it == TR else [u[:1] for u in x]
                r = h[0].astype(BF16).astype(F32)
                e2 = (r - h[0]) * 0.5
                h = [r] + [u + e2 for u in h[1:]]
                x = h if it == TR else [jnp.concatenate([a, u[1:]], axis=0) for a, u in zip(h, x)]
            for g in range(4):
                st(it, A4, g, l, x[g])

    def run_stage(stage, tok):
        kind, nm, Q, l = stage
        if nm == 'K':
            pass_k(Q, l, tok)
        elif nm == 'L':
            pass_l(Q, l, tok)
        elif kind == 'init':
            pass_init(Q, l, tok)
        elif kind == 'final':
            pass_final(Q, l, tok)
        else:
            put_y(Q, l, new_x(Q, l, tok))

    def group(G):
        l, ph, i, lorder = G // 49, G // 7 % 7, cfg['morder'][G % 7], cfg['lorder'][G % 4]
        I, src, dst = [(M3, NN, R3), (M5, PP, R5), (M1, TR, HH), (M4, UP, R4), (M7, UM, R7), (M2, GP, R2),
                       (M6, GM, R6)][ph]
        tmp, tver = TMP[(l * 7 + ph) % 2], l + ph / 8
        fs = [lin([(c, ld(src, f, g, l - 1)) for c, f in AOP[i]]) for g in range(4)]
        w = pltpu.bitcast(t_ref.bitcast(U32)[l, I * 7 + i], BF16)
        n = {}
        for k in lorder:
            op = lin([(c, fs[g]) for c, g in AOP[k]]).astype(BF16)
            n[k] = jnp.dot(op, w[:, k * 16:(k + 1) * 16].reshape(128, 128), preferred_element_type=F32)
        e = [None] * 4
        for k, (f, sg, rt) in FIN.items():
            terms = dict([(k, sg)] + [(x, c) for c, x in rt])
            e[f] = lin([(terms[j], n[j]) for j in lorder if j in terms])
        e = stack(e)
        if i in PRIMED:
            st(tmp, PRIMED.index(i), A4, tver, e)
        else:
            f, sg, rt = FIN[i]
            so = -1 if I == M1 else 1
            terms = [(so * sg, e)] + [(so * c, ld(tmp, PRIMED.index(k), A4, tver)) for c, k in rt]
            if I == M1:
                terms += [(1, ld(it[l % 2], f, A4, l)) for it in (R3, R5)]
            st(dst[l % 2], f, A4, l, lin(terms))
        return [n[k] for k in lorder]

    def rows(r, n):
        return pl.ds(pl.multiple_of(r, HALF), n)

    def top_copy(i):
        return pltpu.make_async_copy(ost_ref.at[jnp.where(i == 1, 2, (i + 1) & 1), pl.ds(HALF, HALF)],
                                     o_hbm.at[rows(jnp.where(i == 1, B - HALF, (i - 2) * TM + HALF), HALF)], sem.at[4])

    def main_body(i, carry):
        enter(i)
        env['ver'] = {}
        copies = [
            pltpu.make_async_copy(x_hbm.at[rows(jnp.minimum(i + 1, nt - 1) * TM, TM)], xin_ref.at[(i + 1) & 3], sem.at[2]),
            top_copy(i),
            pltpu.make_async_copy(ost_ref.at[jnp.where(i == 1, 2, i & 1), pl.ds(0, HALF)],
                                  o_hbm.at[rows((i - 1) * TM, HALF)], sem.at[3])]
        copies[0].start()
        copies[1].start()
        todo = schedule(L, cfg)
        toks = []
        for G in range(49 * L):
            if G == 49 * (L - 1) + 3:
                assert all(stage[3] >= 0 for stage, _ in todo)
                copies[2].start()
            toks += group(G)
            while todo and max(p for p, _ in todo[0][1].values()) < len(toks):
                stage, anchors = todo.pop(0)
                tok = [toks[p][8 * r:8 * r + 8] for _, (p, r) in sorted(anchors.items())]
                run_stage(stage, jnp.concatenate(tok, axis=0).reshape(4, RL, 128))
        assert not todo and all(env['ver'][k] == v + L for k, v in env['first'].items())
        for c in copies:
            c.wait()
        return carry

    def w_start(l, slot):
        for c in range(NC):
            pltpu.make_async_copy(ws_hbm.at[l, :, pl.ds(c * 128, 128)], w_ref.at[slot, c], sem.at[slot]).start()

    def w_wait(slot):
        pltpu.make_async_copy(w_ref.at[slot], w_ref.at[slot], sem.at[slot]).wait()

    def second_block():
        return pltpu.make_async_copy(x_hbm.at[pl.ds(TM, TM)], xin_ref.at[1], sem.at[2])

    def pro_layer(l, carry):
        enter(0)
        slot = l & 1
        wu = w_ref.bitcast(U32).at[slot]
        xb, xu = xb_ref.at[env['z']], xb_ref.bitcast(U32).at[env['z']]
        toks = []
        for m in range(TM // RL):
            rs = pl.ds(m * RL, RL)
            xb[:, rs] = xf_ref[:, rs].astype(BF16)
            for n in range(NC):
                cols = pl.ds(n * 128, 128)
                lhs = pltpu.bitcast(xu[:, pl.ds(m * RL // 2, RL // 2)].reshape(NC * RL // 2, 128), BF16)
                lhs = [jnp.concatenate([lhs[c * RL:(c + 1) * RL] for c in range(h, h + NC // 2)], axis=1)
                       for h in (0, NC // 2)]
                w = pltpu.bitcast(wu[n], BF16)
                y1 = jnp.dot(lhs[0], w[:D // 2], preferred_element_type=F32)
                y2 = y1 + jnp.dot(lhs[1], w[D // 2:], preferred_element_type=F32)
                toks += [y1, y2]
                xf_ref[n, rs] = env['xp'][rs, cols].astype(F32) * (y2 + bp_ref[l, pl.ds(0, 1), cols]) + xf_ref[n, rs]

        buf = env['buf']
        blk = lambda it, f, g: (pl.ds(2 * it, 2), f, g, ROWS)
        dev = lambda k: blk(10, k // 4, k % 4)

        def rnd(x):
            x4 = x.reshape(8, 2, 8, 128)
            r = jnp.concatenate([x4[:, 0], x4[:, 1]], axis=2).astype(BF16).astype(F32)
            return jnp.stack([r[:, :, :128], r[:, :, 128:]], axis=1).reshape(x.shape)

        def w1(q, p, tok):
            v = []
            for Q in range(4):
                r, c = bits(Q, q, p)
                sc = -0.5 * LAM[Q] * LAM[q] * LAM[p]
                wb = pltpu.bitcast(wu[c, pl.ds(r * 64, 64)], BF16).astype(F32).reshape(2, RL, 128)
                v.append(wb * (anchored(sc, tok) if Q == 0 else sc))
            b11, s, t, b22 = v
            tr = b11 + b22
            for F, x in enumerate([tr, b11 - s, b11 + s, tr + (s + t), tr + tr]):
                buf[blk(F, q, p)] = x

        def w2(F, p, tok):
            y = [buf[blk(F, q, p)] for q in range(4)]
            for f, x in enumerate(a_tr(anchored(y[0], tok), *y[1:])):
                buf[blk(5 + F, f, p)] = x

        def w3(I, i, tok):
            b11, s, t, b22 = [lin([(c * C, buf[blk(5 + F, f, p)]) for C, F in BOP_OUT[I] for c, f in BOP[i]])
                              for p in range(4)]
            half = anchored(0.5, tok)
            tr = b11 + b22
            child = I == M1 and i != M1
            if child:
                tr, b11 = tr + buf[dev(0)], b11 + buf[dev(7)]
            r = rnd(tr)
            e2 = (r - tr) * half
            b11 = b11 + e2
            g = (r + (s + t)) * half
            o2, o6 = b11 - s, b11 + s
            out = [tr, o2, r - o6, r - g, r - o2, o6, g]
            if child:
                out = out[:1] + [out[k] + buf[dev(k)] for k in range(1, 7)]
            if I == M1 and i == M1:
                buf[dev(0)], buf[dev(7)] = e2, e2 * 0.5
                for k in range(1, 7):
                    buf[dev(k)] = (rnd(out[k]) - out[k]) * 0.5
            t_ref[l, I * 7 + i] = jnp.concatenate([x.reshape(8, 16, 128) for x in out], axis=1).astype(BF16)

        cost = lambda valu, st_: np.array([valu / 4, st_ * cfg['pa']])
        terms = lambda I, i: len(BOP_OUT[I]) * len(BOP[i])
        groups = [(-1, M1, M1)] + [(0.2 + 0.8 * (j + .5) / 6, M1, j + 1) for j in range(6)]
        for T in (1, 2, 4):
            sel = [(I, i) for I in range(1, 7) for i in range(7) if terms(I, i) == T]
            groups += [((j + .5) / len(sel), I, i) for j, (I, i) in enumerate(sel)]
        passes = [[(cost(29, 10), w1, q, p) for p in range(4) for q in range(4)],
                  [(cost(14, 8), w2, F, p) for p in range(4) for F in range(5)], []]
        for _, I, i in sorted(groups):
            x = (0, 0) if I != M1 else ((38, 16) if i == M1 else (16, 0))
            passes[2].append((cost(8 * (terms(I, i) - 1) + 34 + x[0], 7 + x[1]), w3, I, i))
        span = [(-cfg['l1'], cfg['s1']), (-cfg['l2'], cfg['s2']), (0, 1)]
        seq = sorted((rp + span[si][0] + span[si][1] * j / len(ps), si, j, rp) for si, ps in enumerate(passes)
                     for j in range(len(ps)) for rp in range(8))
        fixed = np.zeros((len(toks), 2)) + cost(24, 0)
        fixed[1::2] += cost(40, 8)
        for o in range(2):
            fixed[(cfg['po'] + o) % 16::16] += cost(16, 16)
        fixed = np.repeat(fixed / 8, 8, axis=0)

        def fill(level):
            where, t, back = {}, 0, np.zeros(2)
            for _, si, j, rp in seq:
                while back.max() > 0 and t < len(fixed) + 64:
                    back = np.maximum(back - (level - fixed[min(t, len(fixed) - 1)]), -cfg['pb'])
                    t += 1
                where[si, j, rp] = divmod(min(t, len(fixed) - 1), 8)
                back = back + passes[si][j][0]
            return where, t
        lo, hi = 4.0, 16.0
        for _ in range(20):
            lo, hi = (lo, (lo + hi) / 2) if fill((lo + hi) / 2)[1] < len(fixed) + cfg['pe'] else ((lo + hi) / 2, hi)
        where = fill(hi)[0]
        for si, ps in enumerate(passes):
            for j, (_, fn, a, b) in enumerate(ps):
                tok = [toks[k][8 * r:8 * r + 8] for k, r in (where[si, j, rp] for rp in range(8))]
                fn(a, b, jnp.concatenate([t for t in tok for _ in range(2)], axis=0).reshape(2, RL, 128))

        pl.when(l + 2 < L)(lambda: w_start(l + 2, slot))
        pl.when(l + 2 == L)(lambda: second_block().start())
        pl.when(l + 1 < L)(lambda: w_wait(1 - slot))
        return carry

    def prologue():
        z_ref[0] = 0
        first = [pltpu.make_async_copy(bs_hbm, bs_ref, sem.at[1]),
                 pltpu.make_async_copy(x_hbm.at[pl.ds(0, HALF)], xin_ref.at[3, pl.ds(0, HALF)], sem.at[2]),
                 pltpu.make_async_copy(x_hbm.at[pl.ds(B - HALF, HALF)], xin_ref.at[3, pl.ds(HALF, HALF)], sem.at[3]),
                 pltpu.make_async_copy(x_hbm.at[pl.ds(HALF, HALF)], xin_ref.at[0, pl.ds(HALF, HALF)], sem.at[4])]
        for c in first:
            c.start()
        w_start(0, 0)
        xb_ref[...] = jnp.zeros(xb_ref.shape, BF16)
        xin_ref[0, pl.ds(0, HALF)] = jnp.zeros((HALF, D), BF16)
        for it in (HH[1], R4[1], R7[1], R2[1], R6[1], C22[0], ZZ[0], DD[2]):
            buf_ref[0, it, A4, A4, ROWS] = jnp.zeros((4, 4, RL, 128), F32)
        first[0].wait()
        beta = [jnp.ones((8, D), F32)]
        for l in range(L):
            bp_ref[l] = jnp.broadcast_to(bs_ref[l:l + 1, :].astype(F32), (8, D))
            beta.append(beta[-1] + bp_ref[l])
        beta = stack(beta[1:])
        for Q in range(4):
            for q in range(4):
                cols = [bits(Q, q, p)[1] * 128 for p in range(4)]
                for p, v in enumerate(scaled([beta[:, :, c:c + 128] for c in cols], Q, q, 1)):
                    bt_ref[:, Q, q, p] = v
        for c in first[1:]:
            c.wait()
        enter(0)
        x0 = env['xp'][...].astype(F32)
        for c in range(NC):
            xf_ref[c, pl.ds(0, TM)] = x0[:, c * 128:(c + 1) * 128]
        for Q in (1, 0):
            pass_init(Q, -1, None)
            pass_l(Q, -1, None)
        w_wait(0)
        w_start(1, 1)
        lax.fori_loop(0, L, pro_layer, 0)
        ost_ref[2] = jnp.concatenate([xf_ref[c, pl.ds(0, TM)] for c in range(NC)], axis=1).astype(BF16)
        second_block().wait()

    def drain():
        enter(nt)
        copies = [top_copy(jnp.int32(nt))]
        copies[0].start()
        for Q in (3, 2):
            pass_k(Q, -1, None)
        for h in range(2):
            for Q in (3, 2):
                pass_final(Q, -1, None, pl.ds(2 * h, 2))
            for j in range(2):
                r = (2 * j + h) * RL
                copies.append(pltpu.make_async_copy(ost_ref.at[nt % 2, pl.ds(r, RL)], o_hbm.at[pl.ds(B - TM + r, RL)],
                                                    sem.at[2 * h + j]))
                copies[-1].start()
        for c in copies:
            c.wait()

    prologue()
    lax.fori_loop(1, nt, main_body, 0)
    drain()


@jax.jit
def pallas_standalone__dcn_v2_cross__recsys_kernel(x0, ws, bs):
    B, D = x0.shape
    L = ws.shape[0]
    assert D == 1024 and L % 2 == 0 and B % TM == 0 and B >= 2 * TM
    cfg = dict(CFG)
    cfg.update(morder=[int(c) - 1 for c in str(cfg['mo'])], lorder=[[int(c) - 1 for c in o] for o in (str(cfg['lo']).split('x') * 4)[:4]])
    any_spec = pl.BlockSpec(memory_space=pl.ANY)
    return pl.pallas_call(
        functools.partial(_kernel, cfg=cfg),
        in_specs=[any_spec] * 3,
        out_specs=any_spec,
        out_shape=jax.ShapeDtypeStruct((B, D), x0.dtype),
        scratch_shapes=[
            pltpu.SMEM((1,), jnp.int32),
            pltpu.VMEM((1, NI, 5, 5, RL + 8, 128), F32),
            pltpu.VMEM((L, 49, 8, 7 * 16, 128), BF16),
            pltpu.VMEM((L, 4, 4, 4, 8, 128), F32),
            pltpu.VMEM((L, 8, D), F32),
            pltpu.VMEM((2, D // 128, D, 128), BF16),
            pltpu.VMEM((D // 128, TM + 8, 128), F32),
            pltpu.VMEM((1, D // 128, TM, 128), BF16),
            pltpu.VMEM((4, TM, D), BF16),
            pltpu.VMEM((3, TM, D), BF16),
            pltpu.VMEM((L, D), BF16),
            pltpu.SemaphoreType.DMA((5,)),
        ],
        compiler_params=pltpu.CompilerParams(vmem_limit_bytes=127 * 1024 * 1024),
    )(x0, ws, bs)
```
